```python
import os as _os
_os.environ.setdefault('JAX_PLATFORMS', 'cpu')
import jax
import jax.numpy as jnp

def _softmax(x, axis=-1):
    return jax.nn.softmax(x, axis=axis)

def _gelu(x):
    return jax.nn.gelu(x, approximate=True)

def _silu(x):
    return jax.nn.silu(x)

def _sigmoid(x):
    return jax.nn.sigmoid(x)

def _layernorm(x, axis=-1, eps=1e-05):
    m = jnp.mean(x, axis=axis, keepdims=True)
    v = jnp.var(x, axis=axis, keepdims=True)
    return (x - m) / jnp.sqrt(v + eps)

def _scatter_add(tgt, idx, src, axis=0):
    return tgt.at[idx].add(src)

def _segment_sum(src, seg, n):
    return jax.ops.segment_sum(src, seg, n)

class _Rng:

    def __init__(self, key):
        self._k = key

    def _next(self):
        self._k, sub = jax.random.split(self._k)
        return sub

    def normal(self, shape):
        return jax.random.normal(self._next(), shape, dtype=jnp.bfloat16)

    def randint(self, lo, hi, shape):
        return jax.random.randint(self._next(), shape, lo, hi, dtype=jnp.int32)

    def uniform(self, shape, lo=0.0, hi=1.0):
        return jax.random.uniform(self._next(), shape, jnp.bfloat16, lo, hi)

    def permutation(self, n):
        return jax.random.permutation(self._next(), n)
kernel_name = 'adaLN_cond__grouped_kv_mqa__mixer_gmlp__prompt'

def setup_inputs():
    _rng = _Rng(jax.random.key(int.from_bytes(__import__("os").urandom(4), "little")))
    _w = lambda a: (lambda t: t.astype(jnp.bfloat16) if jnp.issubdtype(t.dtype, jnp.floating) else t)(jnp.asarray(a))

    def _A_setup():
        B, S, D, H = (1, 2048, 512, 32)
        Dh = D // H
        return {'x': _w((lambda *s: _rng.normal(s) * 0.05)(B, S, D)), 'wq': _w((lambda *s: _rng.normal(s) * 0.05)(D, H * Dh)), 'wk': _w((lambda *s: _rng.normal(s) * 0.05)(D, Dh)), 'wv': _w((lambda *s: _rng.normal(s) * 0.05)(D, Dh)), 'wo': _w((lambda *s: _rng.normal(s) * 0.05)(H * Dh, D))}
    _A_in = _A_setup()

    def _B_setup():
        B, S, D, F = (1, 2048, 512, 1792)
        Fh = F // 2
        return {'x': _w((lambda *s: _rng.normal(s) * 0.05)(B, S, D)), 'w_in': _w((lambda *s: _rng.normal(s) * 0.4)(D, 2 * Fh)), 'w_sp': _w(0.01 * (lambda *s: _rng.normal(s) * 0.4)(S, S)), 'b_sp': _w(1.0 + 0.01 * (lambda *s: _rng.normal(s) * 0.05)(S)), 'w_out': _w((lambda *s: _rng.normal(s) * 0.05)(Fh, D))}
    _B_in = _B_setup()
    return {'A_x': _A_in['x'], 'A_wq': _A_in['wq'], 'A_wk': _A_in['wk'], 'A_wv': _A_in['wv'], 'A_wo': _A_in['wo'], 'B_x': _B_in['x'], 'B_w_in': _B_in['w_in'], 'B_w_sp': _B_in['w_sp'], 'B_b_sp': _B_in['b_sp'], 'B_w_out': _B_in['w_out'], 'c': _w((lambda *s: _rng.normal(s) * 0.05)(1, 512) * 8.0), 'w_mod': _w((lambda *s: _rng.normal(s) * 0.05)(512, 6 * 512) * 512 ** (-0.5) * 8.0)}

def reference(A_x, A_wq, A_wk, A_wv, A_wo, B_x, B_w_in, B_w_sp, B_b_sp, B_w_out, c, w_mod):

    def _A_ref(x, wq, wk, wv, wo):
        B, S, D = x.shape
        H = 32
        Dh = D // H
        q = (lambda x, *d: x.transpose(*d))((x @ wq).reshape(B, S, H, Dh), 0, 2, 1, 3)
        k = x @ wk
        v = x @ wv
        scores = jnp.einsum('bhqd,bkd->bhqk', q, k) * Dh ** (-0.5)
        p = _softmax(scores, axis=-1)
        o = jnp.einsum('bhqk,bkd->bhqd', p, v)
        return (lambda x, *d: x.transpose(*d))(o, 0, 2, 1, 3).reshape(B, S, H * Dh) @ wo

    def _B_ref(x, w_in, w_sp, b_sp, w_out):
        B, S, D = x.shape
        F = w_in.shape[-1]
        Fh = F // 2
        z = _gelu(jnp.einsum('bsd,df->bsf', x, w_in))
        z1 = z[..., :Fh].copy()
        z2 = _layernorm(z[..., Fh:], axis=-1)
        g = jnp.einsum('ts,bsf->btf', w_sp, z2) + b_sp[None, :, None]
        return jnp.einsum('bsf,fd->bsd', z1 * g, w_out)
    x = A_x
    mod = (_silu(c) @ w_mod).reshape(c.shape[0], 6, 1, -1)
    sa, ca, ga, sb, cb, gb = (mod[:, 0].copy(), mod[:, 1].copy(), mod[:, 2].copy(), mod[:, 3].copy(), mod[:, 4].copy(), mod[:, 5].copy())
    h = _layernorm(x, axis=-1) * (1 + ca) + sa
    x = x + ga * _A_ref(h, A_wq, A_wk, A_wv, A_wo)
    h = _layernorm(x, axis=-1) * (1 + cb) + sb
    x = x + gb * _B_ref(h, B_w_in, B_w_sp, B_b_sp, B_w_out)
    return x
```

```python
import math

import jax
import jax.numpy as jnp
from jax import lax
import jax.experimental.pallas as pl
import jax.experimental.pallas.tpu as pltpu

F32 = jnp.float32
BF16 = jnp.bfloat16
U32 = jnp.uint32

S, D, H, DH, F, FH = 2048, 512, 32, 16, 1792, 896
NQ = 512
NT = NQ // 128
KB = 128
NKB = S // KB
EPS = 1e-5
QSCALE = DH ** -0.5 * math.log2(math.e)
SAFE_BOUND = 40.0
NSLOT = 3

NT_DIMS = (((1,), (1,)), ((), ()))


def _layernorm(x):
    m = jnp.mean(x, axis=-1, keepdims=True)
    xc = x - m
    v = jnp.mean(xc * xc, axis=-1, keepdims=True)
    return xc * lax.rsqrt(v + EPS)


def _gelu(x):
    c0 = math.sqrt(2.0 / math.pi)
    c1 = c0 * 0.044715
    hx = 0.5 * x
    return hx + hx * jnp.tanh(x * (c0 + c1 * (x * x)))


def make(nv=(16,), U=4, skew=2, RC=512, RD=512, chains=2, phases='ABCD', flags=None):
    nvs = [nv[kb % len(nv)] for kb in range(NKB)]
    goff = [0]
    for n in nvs:
        goff.append(goff[-1] + n // 8)
    NG = goff[-1]
    NZ = 64 + U * (2 * NG * NT + NKB + 2)

    def kernel(x_hbm, wq_hbm, wkt_hbm, wvt_hbm, wo_hbm, win_hbm, wsp_hbm, bsp_hbm, wout_hbm, c_hbm, wmod_hbm,
               out_hbm,
               x_v, wq_v, wkt_v, wvt_v, wo_v, win_v, wsp_v, bsp_v, wout_v, c_v, wmod_v, out_v,
               zero_s, mod_s, wt_s, qt_s, kf_s, k_s, vt_s, kb_s, qb_s, ot_s, x1_s, z1_s, z2_s, bcol_s,
               sem, osem, *p_s):
        def cp(i, src, dst):
            return pltpu.make_async_copy(src, dst, sem.at[i])

        c_cp = cp(0, c_hbm, c_v)
        wmod_a_cp = cp(1, wmod_hbm.at[:, pl.ds(0, 2 * D)], wmod_v.at[:, pl.ds(0, 2 * D)])
        wq_cp = cp(2, wq_hbm, wq_v)
        wkt_cp = cp(3, wkt_hbm, wkt_v)
        wvt_cp = cp(4, wvt_hbm, wvt_v)
        x_cps = [cp(5 + i, x_hbm.at[pl.ds(i * NQ, NQ)], x_v.at[pl.ds(i * NQ, NQ)]) for i in range(S // NQ)]
        wmod_b_cp = cp(9, wmod_hbm.at[:, pl.ds(2 * D, 4 * D)], wmod_v.at[:, pl.ds(2 * D, 4 * D)])
        wo_cp = cp(10, wo_hbm, wo_v)
        win_cp = cp(11, win_hbm, win_v)
        bsp_cp = cp(12, bsp_hbm, bsp_v)
        wout_cp = cp(13, wout_hbm, wout_v)
        wsp_cp = cp(14, wsp_hbm, wsp_v)
        for d in (c_cp, wq_cp, wkt_cp, wvt_cp, wmod_a_cp, *x_cps):
            d.start()

        def zinit(i, c):
            zero_s[i] = 0
            return c
        lax.fori_loop(0, NZ, zinit, 0)

        wq_cp.wait()
        for i in range(D // 128):
            wt_s[i * 128:(i + 1) * 128, :] = wq_v[:, i * 128:(i + 1) * 128].astype(F32).T.astype(BF16)
        wkt_cp.wait()
        wvt_cp.wait()
        wt_s[D:D + DH, :] = wkt_v[...]
        wt_s[D + DH:D + 2 * DH, :] = wvt_v[...]

        c_cp.wait()
        cf = c_v[...].astype(F32)
        sc = jnp.broadcast_to(cf * jax.nn.sigmoid(cf), (16, D)).astype(BF16)
        wmod_a_cp.wait()
        mod_a = jnp.dot(sc, wmod_v[:, 0:2 * D], preferred_element_type=F32)[0:8]
        sa = mod_a[0:1, 0:D]
        ca1 = 1.0 + mod_a[0:1, D:2 * D]

        qmax = jnp.zeros((1, NQ), F32)
        kmax = jnp.zeros((1, NQ), F32)
        vmax = jnp.zeros((DH, NQ), F32)
        for j in range(S // NQ):
            x_cps[j].wait()
            if j == S // NQ - 1:
                for d in (wmod_b_cp, wo_cp, win_cp, bsp_cp, wout_cp, wsp_cp):
                    d.start()
            cols = slice(j * NQ, (j + 1) * NQ)
            hb = (_layernorm(x_v[cols, :].astype(F32)) * ca1 + sa).astype(BF16)
            r = lax.dot_general(wt_s[...], hb, NT_DIMS, preferred_element_type=F32)
            qb16 = (r[0:D] * QSCALE).astype(BF16)
            qt_s[:, cols] = pltpu.bitcast(qb16, U32)
            qf = qb16.astype(F32)
            q2 = jnp.sum((qf * qf).reshape(H, DH, NQ), axis=1)
            qmax = jnp.maximum(qmax, jnp.max(q2, axis=0, keepdims=True))
            kt = r[D:D + DH].astype(BF16).astype(F32)
            kmax = jnp.maximum(kmax, jnp.sum(kt * kt, axis=0, keepdims=True))
            kf_s[cols, :] = kt.T
            vt = r[D + DH:D + 2 * DH]
            vmax = jnp.maximum(vmax, jnp.abs(vt))
            vt_s[:, cols] = pltpu.bitcast(vt.astype(BF16), U32)

        for g in range(S // 16):
            ev = kf_s[pl.ds(16 * g, 8, stride=2), :]
            od = kf_s[pl.ds(16 * g + 1, 8, stride=2), :]
            k_s[8 * g:8 * g + 8, :] = pltpu.bitcast(jnp.concatenate([ev, od], axis=0).astype(BF16), U32)
            kb, gi = divmod(g, KB // 16)
            first_vpu = (KB - nvs[kb]) // 16
            if gi >= first_vpu:
                for e, val in enumerate((ev, od)):
                    slot = goff[kb] + 2 * (gi - first_vpu) + e
                    for dd in range(DH):
                        kb_s[slot * DH + dd] = jnp.broadcast_to(val[:, dd:dd + 1], (8, 128))

        safe = jnp.logical_and(jnp.max(qmax) * jnp.max(kmax) <= SAFE_BOUND * SAFE_BOUND,
                               jnp.max(vmax) <= 2.0 ** 60)

        def getq(h, j):
            return qt_s[pl.ds(pl.multiple_of(h * 8, 8), 8), pl.ds(pl.multiple_of(j * NQ, NQ), NQ)]

        def puto(h, j, val):
            ot_s[pl.ds(pl.multiple_of(h * DH, DH), DH), pl.ds(pl.multiple_of(j * NQ, NQ), NQ)] = val

        def fast_body(it, carry):
            j = it // (H // U)
            h0 = (it % (H // U)) * U
            ss, half, lsum, acc = {}, {}, {}, {}
            T = U * NKB
            cnt = [0]

            def zero():
                cnt[0] += 1
                return zero_s[cnt[0] % NZ]

            for u in range(U if NG else 0):
                qp = getq(h0 + u, j)
                for e in range(2):
                    qe = pltpu.unpack_elementwise(qp, index=e, packed_dtype=BF16, unpacked_dtype=F32)
                    for i in range(8):
                        qb_s[u, 2 * i + e] = jnp.broadcast_to(qe[i:i + 1, :], (8, NQ))

            def vpu_scores(u, kb, g, n):
                a = [None] * chains
                zk, zq = zero(), zero()
                for dd in range(DH):
                    pr = kb_s[(goff[kb] + g) * DH + dd + zk] * qb_s[u + zq, dd, :, n * 128:(n + 1) * 128]
                    a[dd % chains] = pr if dd < chains else a[dd % chains] + pr
                while len(a) > 1:
                    a = [a[i] + a[i + 1] for i in range(0, len(a), 2)]
                return a[0]

            def addl(u, n, p):
                lsum[u, n] = p if (u, n) not in lsum else lsum[u, n] + p

            def putp(t, i, n, lo, hi):
                p_s[t % NSLOT][0, 8 * i:8 * i + 8, n * 128:(n + 1) * 128] = pltpu.pack_elementwise(
                    [lo, hi], packed_dtype=BF16)

            def soft(t):
                u, kb = divmod(t, NKB)
                ng = nvs[kb] // 8
                nm = (KB - nvs[kb]) // 16
                items = [(g, n) for g in range(ng) for n in range(NT)]
                done = 0
                s = ss.pop(t)
                for i in range(nm):
                    for n in range(NT):
                        lo = jnp.exp2(s[16 * i:16 * i + 8, n * 128:(n + 1) * 128])
                        hi = jnp.exp2(s[16 * i + 8:16 * i + 16, n * 128:(n + 1) * 128])
                        addl(u, n, lo)
                        addl(u, n, hi)
                        putp(t, i, n, lo, hi)
                    while done < (len(items) * (i + 1) + nm - 1) // nm:
                        g, n = items[done]
                        done += 1
                        p = jnp.exp2(vpu_scores(u, kb, g, n))
                        addl(u, n, p)
                        if g % 2 == 0:
                            half[n] = p
                        else:
                            putp(t, nm + g // 2, n, half.pop(n), p)

            zv = {}

            def pv(t):
                u, kb = divmod(t, NKB)
                if kb == 0:
                    zv[u] = zero()
                pb = pltpu.bitcast(p_s[t % NSLOT][zero()], BF16)
                vb = pltpu.bitcast(vt_s[:, pl.ds(pl.multiple_of(kb * KB + zv[u] * 128, 128), KB)], BF16)
                d = jnp.dot(vb, pb, preferred_element_type=F32)
                acc[u] = d if kb == 0 else acc[u] + d
                if kb == NKB - 1:
                    l = jnp.sum(jnp.concatenate([lsum.pop((u, n)) for n in range(NT)], axis=1), axis=0, keepdims=True)
                    puto(h0 + u, j, acc.pop(u) * (1.0 / l))

            for t in range(T + skew):
                if t < T:
                    u, kb = divmod(t, NKB)
                    if kb == 0:
                        q = pltpu.bitcast(getq(h0 + u, j), BF16)
                        zk = zero()
                    kk = pltpu.bitcast(
                        k_s[pl.ds(pl.multiple_of(kb * KB // 2 + zk * 8, 8), (KB - nvs[kb]) // 2), :], BF16)
                    ss[t] = jnp.dot(kk, q, preferred_element_type=F32)
                if 1 <= t <= T:
                    soft(t - 1)
                if t >= skew:
                    pv(t - skew)
            return carry

        def slow_body(it, carry):
            j = it // H
            h = it % H
            q = pltpu.bitcast(getq(h, j), BF16)
            s = jnp.dot(kf_s[...].astype(BF16), q, preferred_element_type=F32)
            p = jnp.exp2(s - jnp.max(s, axis=0, keepdims=True))
            l = jnp.sum(p, axis=0, keepdims=True)
            o = jnp.dot(pltpu.bitcast(vt_s[...], BF16), p.astype(BF16), preferred_element_type=F32)
            puto(h, j, o * (1.0 / l))
            return carry

        if 'B' in phases:
            @pl.when(safe)
            def _():
                lax.fori_loop(0, (S // NQ) * H // U, fast_body, 0)

            @pl.when(jnp.logical_not(safe))
            def _():
                lax.fori_loop(0, (S // NQ) * H, slow_body, 0)
        else:
            ot_s[...] = jnp.zeros(ot_s.shape, F32)

        wmod_b_cp.wait()
        mod_b = jnp.dot(sc, wmod_v[:, 2 * D:6 * D], preferred_element_type=F32)[0:8]
        ga = mod_b[0:1, 0:D]
        sb = mod_b[0:1, D:2 * D]
        cb1 = 1.0 + mod_b[0:1, 2 * D:3 * D]
        gb = mod_b[0:1, 3 * D:4 * D]
        wo_cp.wait()
        win_cp.wait()
        bsp_cp.wait()
        bf = bsp_v[...].astype(F32)
        for i in range(S // 128):
            bcol_s[i * 128:(i + 1) * 128, :] = jnp.broadcast_to(bf[i:i + 1, :], (128, 128)).T
        wout_cp.wait()
        wsp_cp.wait()

        h2 = {}

        def c_front(i):
            rows = slice(i * RC, (i + 1) * RC)
            o = ot_s[:, rows].T.astype(BF16)
            x1 = x_v[rows, :].astype(F32) + ga * jnp.dot(o, wo_v[...], preferred_element_type=F32)
            x1_s[rows, :] = x1
            h2[i] = (_layernorm(x1) * cb1 + sb).astype(BF16)

        def c_back(i):
            rows = slice(i * RC, (i + 1) * RC)
            hb = h2.pop(i)
            z2 = _gelu(jnp.dot(hb, win_v[:, FH:F], preferred_element_type=F32))
            z2_s[rows, :] = _layernorm(z2).astype(BF16)
            z1 = _gelu(jnp.dot(hb, win_v[:, 0:FH], preferred_element_type=F32))
            z1_s[rows, :] = z1.astype(BF16)

        nc = S // RC
        for i in range(nc + 1):
            if i < nc:
                c_front(i)
            if i >= 1:
                c_back(i - 1)

        ys = {}

        def d_front(i):
            rows = slice(i * RD, (i + 1) * RD)
            g = jnp.dot(wsp_v[rows, :], z2_s[...], preferred_element_type=F32)
            b = bcol_s[rows, :]
            g = g + jnp.concatenate([b] * (FH // 128), axis=1)
            ys[i] = (z1_s[rows, :].astype(F32) * g).astype(BF16)

        def out_cp(i):
            rows = pl.ds(i * RD, RD)
            return pltpu.make_async_copy(out_v.at[rows], out_hbm.at[rows], osem.at[i])

        def d_back(i):
            rows = slice(i * RD, (i + 1) * RD)
            y = jnp.dot(ys.pop(i), wout_v[...], preferred_element_type=F32)
            out_v[rows, :] = (x1_s[rows, :] + gb * y).astype(BF16)
            out_cp(i).start()

        nd = S // RD
        for i in range(nd + 1):
            if i < nd:
                d_front(i)
            if i >= 1:
                d_back(i - 1)
        for i in range(nd):
            out_cp(i).wait()

    scratch = [
        pltpu.VMEM((S, D), BF16),
        pltpu.VMEM((D, D), BF16),
        pltpu.VMEM((DH, D), BF16),
        pltpu.VMEM((DH, D), BF16),
        pltpu.VMEM((D, D), BF16),
        pltpu.VMEM((D, F), BF16),
        pltpu.VMEM((S, S), BF16),
        pltpu.VMEM((16, 128), BF16),
        pltpu.VMEM((FH, D), BF16),
        pltpu.VMEM((1, D), BF16),
        pltpu.VMEM((D, 6 * D), BF16),
        pltpu.VMEM((S, D), BF16),
        pltpu.SMEM((NZ,), jnp.int32),
        pltpu.VMEM((8, 6 * D), F32),
        pltpu.VMEM((D + 2 * DH, D), BF16),
        pltpu.VMEM((D // 2, S), U32),
        pltpu.VMEM((S, DH), F32),
        pltpu.VMEM((S // 2, DH), U32),
        pltpu.VMEM((DH // 2, S), U32),
        pltpu.VMEM((max(NG, 1) * DH, 8, 128), F32),
        pltpu.VMEM((U, DH, 8, NQ), F32),
        pltpu.VMEM((D, S), F32),
        pltpu.VMEM((S, D), F32),
        pltpu.VMEM((S, FH), BF16),
        pltpu.VMEM((S, FH), BF16),
        pltpu.VMEM((S, 128), F32),
        pltpu.SemaphoreType.DMA((15,)),
        pltpu.SemaphoreType.DMA((S // RD,)),
    ] + [pltpu.VMEM((1, KB // 2, NQ), U32)] * NSLOT

    def fused(A_x, A_wq, A_wk, A_wv, A_wo, B_x, B_w_in, B_w_sp, B_b_sp, B_w_out, c, w_mod):
        del B_x
        out = pl.pallas_call(
            kernel,
            out_shape=jax.ShapeDtypeStruct((S, D), BF16),
            in_specs=[pl.BlockSpec(memory_space=pl.ANY)] * 11,
            out_specs=pl.BlockSpec(memory_space=pl.ANY),
            scratch_shapes=scratch,
            compiler_params=pltpu.CompilerParams(vmem_limit_bytes=110 * 1024 * 1024, flags=flags),
        )(A_x.reshape(S, D), A_wq, A_wk.T, A_wv.T, A_wo, B_w_in, B_w_sp, B_b_sp.reshape(16, 128), B_w_out,
          c, w_mod)
        return out.reshape(1, S, D)

    return fused


_fused = make(nv=(16,), U=2)


@jax.jit
def pallas_adaLN_cond__grouped_kv_mqa__mixer_gmlp__prompt_kernel(
    A_x, A_wq, A_wk, A_wv, A_wo, B_x, B_w_in, B_w_sp, B_b_sp, B_w_out, c, w_mod,
):
    return _fused(A_x, A_wq, A_wk, A_wv, A_wo, B_x, B_w_in, B_w_sp, B_b_sp, B_w_out, c, w_mod)
```

```python
import bisect
import math

import jax
import jax.numpy as jnp
from jax import lax
import jax.experimental.pallas as pl
import jax.experimental.pallas.tpu as pltpu

F32 = jnp.float32
BF16 = jnp.bfloat16
U32 = jnp.uint32

S, D, H, DH, F, FH = 2048, 512, 32, 16, 1792, 896
NQ = 512
NT = NQ // 128
NJ = S // NQ
KB = 128
NKB = S // KB
EPS = 1e-5
QSCALE = DH ** -0.5 * math.log2(math.e)
SAFE_BOUND = 64.0
NSLOT = 4
NZ = 64

NT_DIMS = (((1,), (1,)), ((), ()))

STRASSEN = [
    ([((1, 0), 1), ((1, 1), 1)], [((0, 0), 1)], [((1, 0), 1), ((1, 1), -1)]),
    ([((1, 1), 1)], [((1, 0), 1), ((0, 0), -1)], [((0, 0), 1), ((1, 0), 1)]),
    ([((0, 0), 1), ((1, 1), 1)], [((0, 0), 1), ((1, 1), 1)], [((0, 0), 1), ((1, 1), 1)]),
    ([((0, 0), 1), ((0, 1), 1)], [((1, 1), 1)], [((0, 0), -1), ((0, 1), 1)]),
    ([((0, 1), 1), ((1, 1), -1)], [((1, 0), 1), ((1, 1), 1)], [((0, 0), 1)]),
    ([((0, 0), 1)], [((0, 1), 1), ((1, 1), -1)], [((0, 1), 1), ((1, 1), 1)]),
    ([((1, 0), 1), ((0, 0), -1)], [((0, 0), 1), ((0, 1), 1)], [((1, 1), 1)]),
]
CLASSIC = [([((i, k), 1)], [((k, j), 1)], [((i, j), 1)]) for j in range(2) for i in (1, 0) for k in range(2)]


def _lincomb(terms, get):
    acc = None
    for p, s in sorted(terms, key=lambda t: -t[1]):
        v = get(p)
        if acc is None:
            acc = v if s > 0 else -v
        else:
            acc = acc + v if s > 0 else acc - v
    return acc


def _touches_later(alg, i, p):
    return any(p == q for _, _, c in alg[i + 1:] for q, _ in c)


def _ln_cols(x):
    xc = x - jnp.mean(x, axis=0, keepdims=True)
    v = jnp.mean(xc * xc, axis=0, keepdims=True)
    return xc * lax.rsqrt(v + EPS)


def _gelu_of_half(hx):
    c0 = 2.0 * math.sqrt(2.0 / math.pi)
    c1 = c0 * 4.0 * 0.044715
    return hx + hx * jnp.tanh(hx * (c0 + c1 * (hx * hx)))


def _pack(x):
    return pltpu.bitcast(x.astype(BF16), U32)


def _pack2(x):
    return pltpu.pack_elementwise([x[0:8], x[8:16]], packed_dtype=BF16)


def _unpack(w):
    return pltpu.bitcast(w, BF16)


def _lanes(col, n):
    return jnp.concatenate([col] * (n // 128), axis=1)


def make(nv=(16, 16, 16, 32), U=8, skew=2, chains=2, phase=0.0, phases='B', flags=None, win_alg='s', sp_lv=2,
         out_blocks=((1024, 512), (1536, 512), (0, 512), (512, 256), (768, 128), (896, 128)), scopes=False, qstep=4, xwait=10, xlast=26, xcuts=(512, 768), dorder=0, cpos=4, biters=None,
         win_ord=(1, 0, 2, 5, 6, 3, 4), out_ord=(5, 3, 2, 6, 0, 1, 4), in_ord=(5, 3, 2, 6, 0, 1, 4), back_at=(1, 1)):
    nvs = [nv[kb % len(nv)] for kb in range(NKB)]
    goff, moff = [0], [0]
    for n in nvs:
        goff.append(goff[-1] + n // 8)
        moff.append(moff[-1] + (KB - n) // 8)
    NG, NM = goff[-1], moff[-1]
    assert all(n % 16 == 0 for n in nvs) and NM % 2 == 0 and NG % 2 == 0 and NG <= NZ and U <= NZ
    qoff = [(m + 1) // 2 for m in moff]
    WIN = [STRASSEN[i] for i in win_ord] if win_alg == 's' else CLASSIC

    def kernel(x_hbm, wq_hbm, wkt_hbm, wvt_hbm, wo_hbm, win_hbm, wsp_hbm, bsp_hbm, wout_hbm, c_hbm, wmod_hbm,
               out_hbm,
               x_v, wq_v, wkt_v, wvt_v, wo_v, win_v, wsp_v, wout_v, wmod_v, out_v,
               zero_s, mod_s, wt_s, qt_s, qf0_s, qf1_s, kf_s, k_s, vt_s, kb_s, xt_s, ot_s, wot_s, wint_s, wina_s,
               woutt_s, h2_s, z1_s, z2_s, g_s, y_s, wsum_s, macc_s, p0_s, p1_s, p2_s, p3_s, b_s, bsp_v, c_v,
               sem, osem):
        p_s = (p0_s, p1_s, p2_s, p3_s)
        qf_s = (qf0_s, qf1_s)
        import contextlib
        stack = contextlib.ExitStack()

        def mark(name):
            if scopes:
                stack.close()
                if name:
                    stack.enter_context(jax.named_scope(name))
        mark('A0_start')

        def cp(i, src, dst):
            return pltpu.make_async_copy(src, dst, sem.at[i])

        c_cp = cp(0, c_hbm, c_v)
        wmod_a_cp = cp(1, wmod_hbm.at[:, pl.ds(0, 2 * D)], wmod_v.at[:, pl.ds(0, 2 * D)])
        wq_cp = cp(2, wq_hbm, wq_v)
        wkt_cp = cp(3, wkt_hbm, wkt_v)
        wvt_cp = cp(4, wvt_hbm, wvt_v)
        x_cps = [cp(5 + i, x_hbm.at[pl.ds(lo, hi - lo)], x_v.at[pl.ds(lo, hi - lo)])
                 for i, (lo, hi) in enumerate(zip((0, *xcuts), (*xcuts, S)))]
        wmod_b_cp = cp(9, wmod_hbm.at[:, pl.ds(2 * D, 4 * D)], wmod_v.at[:, pl.ds(2 * D, 4 * D)])
        wo_cp = cp(10, wo_hbm, wo_v)
        win_cp = cp(11, win_hbm, win_v)
        bsp_cp = cp(12, bsp_hbm, bsp_v)
        wout_cp = cp(13, wout_hbm, wout_v)
        wsp_cp = cp(14, wsp_hbm, wsp_v)
        for d in ((c_cp, x_cps[0], wmod_a_cp, wkt_cp, wvt_cp, wq_cp, *x_cps[1:]),
                  (c_cp, wmod_a_cp, x_cps[0], wkt_cp, wvt_cp, wq_cp, *x_cps[1:]),
                  (c_cp, wkt_cp, wvt_cp, wq_cp, x_cps[0], wmod_a_cp, *x_cps[1:]))[dorder]:
            d.start()

        def zinit(i, c):
            zero_s[i] = 0
            return c
        lax.fori_loop(0, NZ, zinit, 0)

        def transpose_into(dst, src, rows, cols, at=0):
            for i in range(cols // 128):
                dst[0, at + i * 64:at + (i + 1) * 64, :] = pltpu.bitcast(src[0:rows, i * 128:(i + 1) * 128].T, U32)

        def column_table(i, row):
            mod_s[i] = jnp.broadcast_to(row, (128, D)).T

        c_cp.wait()
        cf = c_v[...].astype(F32)
        sc = jnp.broadcast_to(cf * jax.nn.sigmoid(cf), (16, D)).astype(BF16)

        xn = {}
        bounds = [jnp.zeros((8, 128), F32), jnp.zeros((1, 128), F32), jnp.zeros((DH, 128), F32)]

        def a_norm(n):
            cols = slice(n * 128, (n + 1) * 128)
            xt = x_v[cols, :].T.astype(F32)
            xt_s[:, cols] = xt
            xn[n] = _ln_cols(xt)

        def a_proj(n, lo, hi):
            cols = slice(n * 128, (n + 1) * 128)
            if xn[n].dtype == F32:
                xn[n] = (xn[n] * mod_s[1] + mod_s[0]).astype(BF16)
            r = jnp.dot(_unpack(wt_s[zero_s[n], 8 * lo:8 * hi, :]), xn[n], preferred_element_type=F32)
            for i in range(max(lo, 2), hi):
                qf = r[(i - lo) * DH:(i - lo + 1) * DH] * QSCALE
                qt_s[(i - 2) * 8:(i - 1) * 8, cols] = _pack2(qf)
                bounds[0] = jnp.maximum(bounds[0], qf[0:8] * qf[0:8] + qf[8:16] * qf[8:16])
            if lo > 0:
                return
            kt = r[0:DH].astype(BF16).astype(F32)
            bounds[1] = jnp.maximum(bounds[1], jnp.sum(kt * kt, axis=0, keepdims=True))
            kf_s[cols, :] = kt.T
            bounds[2] = jnp.maximum(bounds[2], jnp.abs(r[DH:2 * DH]))
            vt_s[:, cols] = _pack(r[DH:2 * DH])
            for i in range(KB // 16):
                a1, a2 = (kf_s[pl.ds(n * KB + 16 * i + e, 8, stride=2), :] for e in range(2))
                if i < (KB - nvs[n]) // 16:
                    k_s[8 * (qoff[n] + i):8 * (qoff[n] + i + 1), :] = _pack(jnp.concatenate([a1, a2], axis=0))
                    continue
                g = goff[n] // 2 + i - (KB - nvs[n]) // 16
                for dd in range(8):
                    a11, a12, a21, a22 = (jnp.broadcast_to(a[:, e:e + 1], (8, 128))
                                          for a in (a1, a2) for e in (2 * dd, 2 * dd + 1))
                    for m, v in enumerate((a11 + a22, a21 + a22, a11, a22, a11 + a12, a21 - a11, a12 - a22)):
                        kb_s[g * 56 + m * 8 + dd] = v

        x_cps[0].wait()
        mark('A1_proj')
        for n in range(xcuts[0] // 128):
            a_norm(n)
        mark('A2_waitmod')
        wmod_a_cp.wait()
        mark('A3_mod')
        mod_a = jnp.dot(sc, wmod_v[:, 0:2 * D], preferred_element_type=F32)
        column_table(0, mod_a[0:1, 0:D])
        column_table(1, 1.0 + mod_a[0:1, D:2 * D])
        mark('A4_waitwq')
        wq_cp.wait()
        mark('A5_wq')
        transpose_into(wt_s, wq_v, D, D, at=DH)
        wkt_cp.wait()
        wvt_cp.wait()
        wt_s[0, 0:8, :] = _pack2(wkt_v[...].astype(F32))
        wt_s[0, 8:16, :] = pltpu.bitcast(wvt_v[...], U32)
        mark('A6_waitx1')
        x_cps[1].wait()
        mark('A7_first')
        ends = [c // 128 - 1 for c in xcuts[1:]] + [NKB - 1]
        for n in range(NKB):
            if n >= xcuts[0] // 128:
                a_norm(n)
            cut = xwait if n < NKB - 2 else xlast
            if n + 1 in ends:
                a_proj(n, 0, cut)
            elif n in ends:
                a_proj(n, 0, 2)
                if n < NKB - 1:
                    x_cps[2 + ends.index(n)].wait()
                if n == ends[-2]:
                    for d in (wo_cp, wmod_b_cp, win_cp, bsp_cp, wout_cp, wsp_cp):
                        d.start()
                a_proj(n - 1, cut, H + 2)
                a_proj(n, 2, H + 2)
            else:
                a_proj(n, 0, H + 2)
        qmax, kmax, vmax = bounds

        safe = jnp.logical_and(
            jnp.max(jnp.sum(qmax, axis=0, keepdims=True)) * jnp.max(kmax) <= SAFE_BOUND * SAFE_BOUND,
            jnp.max(vmax) <= 2.0 ** 40)

        mark('B_att')
        def getq(h, j):
            if isinstance(h, int) and isinstance(j, int):
                return qt_s[h * 8:(h + 1) * 8, j * NQ:(j + 1) * NQ]
            return qt_s[pl.ds(pl.multiple_of(h * 8, 8), 8), pl.ds(pl.multiple_of(j * NQ, NQ), NQ)]

        def puto(h, j, val):
            if isinstance(h, int) and isinstance(j, int):
                ot_s[h * 8:(h + 1) * 8, j * NQ:(j + 1) * NQ] = _pack(val)
                return
            ot_s[pl.ds(pl.multiple_of(h * 8, 8), 8), pl.ds(pl.multiple_of(j * NQ, NQ), NQ)] = _pack(val)

        def query_table(slot, h, j):
            lo, hi = (pltpu.unpack_elementwise(getq(h, j), index=e, packed_dtype=BF16, unpacked_dtype=F32)
                      for e in range(2))
            for m in range(NT // 2):
                b11, b12 = lo[:, 256 * m:256 * m + 128], lo[:, 256 * m + 128:256 * m + 256]
                b21, b22 = hi[:, 256 * m:256 * m + 128], hi[:, 256 * m + 128:256 * m + 256]
                for i, v in enumerate((b11 + b22, b11, b12 - b22, b21 - b11, b22, b11 + b12, b21 + b22)):
                    qf_s[slot][0, 8 * i:8 * i + 8, m * 128:(m + 1) * 128] = v

        def pv_tile(t):
            u, kb = divmod(t, NKB)
            pb = _unpack(p_s[t % NSLOT][zero_s[t % NZ]])
            vb = _unpack(vt_s[:, pl.ds(pl.multiple_of(kb * KB + zero_s[u % NZ] * 128, 128), KB)])
            return jnp.dot(vb, pb, preferred_element_type=F32)

        def finish(h, j, acc, lsum):
            puto(h, j, acc * (1.0 / jnp.sum(lsum, axis=0, keepdims=True)))

        def fast_body(it, carry):
            j = it // (H // U)
            h0 = (it % (H // U)) * U
            scores, pend, lsum, acc, done = {}, {}, {}, {}, {}
            items = [(g, o) for g in range(0, NG, 2) for o in range(4)]
            weights = [0]
            for _, o in items:
                weights.append(weights[-1] + (31, 31, 33, 18)[o])
            memo = {}

            def vpu_scores(u, g, o):
                zk = zero_s[u]
                zq = zero_s[g]

                def prod(i):
                    ks = [kb_s[(g // 2) * 56 + i * 8 + dd + zk] for dd in range(8)]
                    res = []
                    for m in range(2):
                        a = [None] * chains
                        for dd in range(8):
                            row = qf_s[u % 2][zq, 8 * i + dd:8 * i + dd + 1, m * 128:(m + 1) * 128]
                            pr = ks[dd] * jnp.broadcast_to(row, (8, 128))
                            a[dd % chains] = pr if dd < chains else a[dd % chains] + pr
                        while len(a) > 1:
                            a = [a[e] + a[e + 1] for e in range(0, len(a), 2)]
                        res.append(a[0])
                    return res

                def add(a, b):
                    return [x + y for x, y in zip(a, b)]

                def sub(a, b):
                    return [x - y for x, y in zip(a, b)]

                if o == 0:
                    memo[3], memo[5] = prod(2), prod(4)
                    return g, 1, add(memo[3], memo[5])
                if o == 1:
                    memo[2], memo[4] = prod(1), prod(3)
                    return g + 1, 0, add(memo[2], memo[4])
                if o == 2:
                    part = add(sub(memo.pop(4), memo.pop(5)), prod(6))
                    memo[1] = prod(0)
                    return g, 0, add(part, memo[1])
                return g + 1, 1, add(add(sub(memo.pop(3), memo.pop(2)), memo.pop(1)), prod(5))

            def emit(u, kb, r, n, s):
                p = jnp.exp2(s)
                lsum[u, n] = p if (u, n) not in lsum else lsum[u, n] + p
                t = u * NKB + kb
                if (t, r ^ 1, n) in pend:
                    o = pend.pop((t, r ^ 1, n))
                    p_s[t % NSLOT][0, 8 * (r // 2):8 * (r // 2) + 8, n * 128:(n + 1) * 128] = (
                        pltpu.pack_elementwise([p, o] if r % 2 == 0 else [o, p], packed_dtype=BF16))
                else:
                    pend[t, r, n] = p

            def do_items(u, upto):
                while done.get(u, 0) < upto:
                    g, n, ss = vpu_scores(u, *items[done.get(u, 0)])
                    done[u] = done.get(u, 0) + 1
                    kb = bisect.bisect_right(goff, g) - 1
                    for m, s in enumerate(ss):
                        emit(u, kb, (KB - nvs[kb]) // 8 + g - goff[kb], 2 * m + n, s)

            def soft(t):
                u, kb = divmod(t, NKB)
                s = scores.pop(t)
                for i in range(qoff[kb], qoff[kb + 1]):
                    for n in range(NT):
                        for e in range(2):
                            r0 = 16 * (i - qoff[kb]) + 8 * e
                            kb2 = bisect.bisect_right(moff, 2 * i + e) - 1
                            emit(u, kb2, 2 * i + e - moff[kb2], n, s[r0:r0 + 8, n * 128:(n + 1) * 128])
                        if (n + 1) % (NT // cpos) == 0:
                            do_items(u, min(len(items), bisect.bisect_left(
                                weights, (i + (n + 1) / NT + phase) / (NM // 2) * weights[-1] - 1e-9)))
                do_items(u, (goff[kb + 1] + 1) // 2 * 4)

            T = U * NKB
            prev = (it + NJ * H // U - 1) % (NJ * H // U)
            acc[-1], lsum[-1] = carry
            for t in range(T):
                u, kb = divmod(t, NKB)
                if kb == 0:
                    q = _unpack(getq(h0 + u, j))
                kk = k_s[pl.ds(pl.multiple_of(8 * qoff[kb] + zero_s[u] * 8, 8), 8 * (qoff[kb + 1] - qoff[kb])), :]
                scores[t] = jnp.dot(_unpack(kk), q, preferred_element_type=F32)
                if kb == qstep and u + 1 < U:
                    query_table((u + 1) % 2, h0 + u + 1, j)
                elif kb == qstep:
                    nxt = jnp.minimum(it + 1, NJ * H // U - 1)
                    query_table(0, (nxt % (H // U)) * U, nxt // (H // U))
                if t >= 1:
                    soft(t - 1)
                u, kb = divmod(t - skew, NKB)
                d = pv_tile(t - skew)
                acc[u] = d if kb == 0 else acc[u] + d
                if kb == NKB - 1 and u < 0:
                    finish((prev % (H // U)) * U + U - 1, prev // (H // U), acc[u], lsum[u])
                elif kb == NKB - 1:
                    finish(h0 + u, j, acc[u], jnp.concatenate([lsum[u, n] for n in range(NT)], axis=1))
            soft(T - 1)
            return acc[U - 1], jnp.concatenate([lsum[U - 1, n] for n in range(NT)], axis=1)

        def slow_body(it, carry):
            j = it // H
            h = it % H
            s = jnp.dot(kf_s[...].astype(BF16), _unpack(getq(h, j)), preferred_element_type=F32)
            p = jnp.exp2(s - jnp.max(s, axis=0, keepdims=True))
            l = jnp.sum(p, axis=0, keepdims=True)
            o = jnp.dot(_unpack(vt_s[...]), p.astype(BF16), preferred_element_type=F32)
            puto(h, j, o * (1.0 / l))
            return carry

        if 'B' in phases:
            @pl.when(safe)
            def _():
                query_table(0, 0, 0)
                for t in range(-skew, 0):
                    p_s[t % NSLOT][...] = jnp.zeros(p_s[0].shape, U32)
                acc, lsum = lax.fori_loop(0, biters or NJ * H // U, fast_body,
                                          (jnp.zeros((DH, NQ), F32), jnp.ones((8, NQ), F32)))
                for t in range(-skew, 0):
                    acc = acc + pv_tile(t)
                finish(H - 1, NJ - 1, acc, lsum)

            @pl.when(jnp.logical_not(safe))
            def _():
                lax.fori_loop(0, NJ * H, slow_body, 0)
        else:
            ot_s[...] = jnp.zeros(ot_s.shape, U32)

        mark('C0_prep')
        for d in (wo_cp, wmod_b_cp, win_cp, bsp_cp, wout_cp, wsp_cp):
            d.wait()
        transpose_into(wot_s, wo_v, D, D)
        for i in range(3):
            row = jnp.dot(sc, wmod_v[:, (2 + i) * D:(3 + i) * D], preferred_element_type=F32)[0:1]
            column_table(2 + i, (row, 0.5 * row, 0.5 + 0.5 * row)[i])
        b_s[...] = bsp_v[...].astype(F32)

        mark('C1_wo')
        for j in range(NJ):
            cols = slice(j * NQ, (j + 1) * NQ)
            a = jnp.dot(_unpack(wot_s[zero_s[j]]), _unpack(ot_s[:, cols]), preferred_element_type=F32)
            x1 = xt_s[:, cols] + _lanes(mod_s[2], NQ) * a
            xt_s[:, cols] = x1
            h2_s[:, cols] = _ln_cols(x1) * _lanes(mod_s[4], NQ) + _lanes(mod_s[3], NQ)

        mark('C2_win')
        transposed = set()

        def win_block(p):
            rows, cols = slice(p[0] * FH, (p[0] + 1) * FH), slice(p[1] * 256, (p[1] + 1) * 256)
            if p not in transposed:
                transposed.add(p)
                wint_s[rows, cols] = win_v[cols, rows].T.astype(F32)
            return wint_s[rows, cols]

        for pair in range(NJ // 2):
            seen = set()
            for i, (at, bt, ct) in enumerate(WIN):
                if pair == 0:
                    wina_s[i] = _pack(_lincomb(at, win_block))
                b = _lincomb(bt, lambda p: h2_s[p[0] * 256:(p[0] + 1) * 256,
                                                (2 * pair + p[1]) * NQ:(2 * pair + p[1] + 1) * NQ])
                m = jnp.dot(_unpack(wina_s[i]), b.astype(BF16), preferred_element_type=F32)
                for p, sg in ct:
                    dst = z2_s if p[0] else z1_s
                    cols = slice((2 * pair + p[1]) * NQ, (2 * pair + p[1] + 1) * NQ)
                    if p in seen:
                        val = dst[:, cols] + m if sg > 0 else dst[:, cols] - m
                    else:
                        seen.add(p)
                        val = m if sg > 0 else -m
                    if not _touches_later(WIN, i, p):
                        val = _gelu_of_half(val)
                        if p[0]:
                            val = _ln_cols(val)
                    dst[:, cols] = val

        mark('D')
        def out_cp(i):
            rows = pl.ds(*out_blocks[i])
            return pltpu.make_async_copy(out_v.at[rows], out_hbm.at[rows], osem.at[i])

        def d_back(i):
            if i == 0:
                transpose_into(woutt_s, wout_v, FH, D)
                column_table(5, jnp.dot(sc, wmod_v[:, 5 * D:6 * D], preferred_element_type=F32)[0:1])
            cols = slice(out_blocks[i][0], out_blocks[i][0] + out_blocks[i][1])
            y = jnp.dot(_unpack(woutt_s[zero_s[i]]), _unpack(y_s[:, cols]), preferred_element_type=F32)
            out_v[cols, :] = (xt_s[:, cols] + _lanes(mod_s[5], out_blocks[i][1]) * y).astype(BF16).T
            out_cp(i).start()

        mb, kb_ = FH // 4, S // 4

        def gate(blk, val):
            rows = slice(blk[0] * mb, (blk[0] + 1) * mb)
            cols = slice(blk[1] * kb_, (blk[1] + 1) * kb_)
            bias = jnp.concatenate([b_s[i:i + 1, :] for i in range(4 * blk[1], 4 * blk[1] + 4)], axis=1)
            y_s[blk[0] * mb // 2:(blk[0] + 1) * mb // 2, cols] = _pack(z1_s[rows, cols] * (val + bias))

        def getz(p):
            return z2_s[p[0] * mb:(p[0] + 1) * mb, p[1] * kb_:(p[1] + 1) * kb_]

        def getw(p):
            return wsp_v[p[1] * kb_:(p[1] + 1) * kb_, p[0] * kb_:(p[0] + 1) * kb_]

        outer = [STRASSEN[i] for i in out_ord] if sp_lv >= 1 else CLASSIC
        inner = [STRASSEN[i] for i in in_ord] if sp_lv >= 2 else CLASSIC
        seen = set()
        nback = 0
        for oi, (a1, b1, c1) in enumerate(outer):
            if len(b1) > 1:
                for r in range(2):
                    for cc in range(2):
                        wsum_s[oi % 2, r * kb_:(r + 1) * kb_, cc * kb_:(cc + 1) * kb_] = _lincomb(
                            b1, lambda p: getw((2 * p[0] + cc, 2 * p[1] + r)).astype(F32))
            seen2 = set()
            for ii, (a2, b2, c2) in enumerate(inner):
                a = _lincomb([((2 * p1[0] + p2[0], 2 * p1[1] + p2[1]), s1 * s2) for p1, s1 in a1 for p2, s2 in a2],
                             getz).astype(BF16)
                if len(b1) > 1:
                    b = _lincomb(b2, lambda p: wsum_s[oi % 2, p[1] * kb_:(p[1] + 1) * kb_,
                                                      p[0] * kb_:(p[0] + 1) * kb_]).astype(BF16)
                else:
                    p1 = b1[0][0]
                    if len(b2) > 1:
                        b = _lincomb(b2, lambda p: getw((2 * p1[0] + p[0], 2 * p1[1] + p[1])).astype(F32)).astype(BF16)
                    else:
                        b = getw((2 * p1[0] + b2[0][0][0], 2 * p1[1] + b2[0][0][1]))
                m = lax.dot_general(a, b, NT_DIMS, preferred_element_type=F32)
                for p, sg in c2:
                    sl = (slice(p[0] * mb, (p[0] + 1) * mb), slice(p[1] * kb_, (p[1] + 1) * kb_))
                    if p in seen2:
                        val = macc_s[sl] + m if sg > 0 else macc_s[sl] - m
                    else:
                        seen2.add(p)
                        val = m if sg > 0 else -m
                    if _touches_later(inner, ii, p):
                        macc_s[sl] = val
                        continue
                    for p1, s1 in c1:
                        blk = (2 * p1[0] + p[0], 2 * p1[1] + p[1])
                        gl = (slice(blk[0] * mb, (blk[0] + 1) * mb), slice(blk[1] * kb_, (blk[1] + 1) * kb_))
                        if blk in seen:
                            tot = g_s[gl] + val if s1 > 0 else g_s[gl] - val
                        else:
                            seen.add(blk)
                            tot = val if s1 > 0 else -val
                        if _touches_later(outer, oi, p1):
                            g_s[gl] = tot
                        else:
                            gate(blk, tot)
                half = out_blocks[0][0] // (S // 2)
                half_done = not any(q[1] == half for _, _, c in outer[oi:] for q, _ in c)
                if half_done and nback < 2 and ii == back_at[nback]:
                    d_back(nback)
                    nback += 1
        while nback < len(out_blocks):
            d_back(nback)
            nback += 1
        mark('E_tail')
        for i in range(len(out_blocks)):
            out_cp(i).wait()
        mark(None)

    scratch = [
        pltpu.VMEM((S, D), BF16),
        pltpu.VMEM((D, D), BF16),
        pltpu.VMEM((DH, D), BF16),
        pltpu.VMEM((DH, D), BF16),
        pltpu.VMEM((D, D), BF16),
        pltpu.VMEM((D, F), BF16),
        pltpu.VMEM((S, S), BF16),
        pltpu.VMEM((FH, D), BF16),
        pltpu.VMEM((D, 6 * D), BF16),
        pltpu.VMEM((S, D), BF16),
        pltpu.SMEM((NZ,), jnp.int32),
        pltpu.VMEM((6, D, 128), F32),
        pltpu.VMEM((1, D // 2 + DH, D), U32),
        pltpu.VMEM((D // 2, S), U32),
        *[pltpu.VMEM((1, 64, NQ // 2), F32)] * 2,
        pltpu.VMEM((S, DH), F32),
        pltpu.VMEM((S // 2, DH), U32),
        pltpu.VMEM((DH // 2, S), U32),
        pltpu.VMEM((max(NG, 2) // 2 * 56, 8, 128), F32),
        pltpu.VMEM((D, S), F32),
        pltpu.VMEM((D // 2, S), U32),
        pltpu.VMEM((1, D // 2, D), U32),
        pltpu.VMEM((F, D), F32),
        pltpu.VMEM((len(WIN), FH // 2, 256), U32),
        pltpu.VMEM((1, D // 2, FH), U32),
        pltpu.VMEM((D, S), F32),
        pltpu.VMEM((FH, S), F32),
        pltpu.VMEM((FH, S), F32),
        pltpu.VMEM((FH, S), F32),
        pltpu.VMEM((FH // 2, S), U32),
        pltpu.VMEM((2, S // 2, S // 2), F32),
        pltpu.VMEM((FH // 2, S // 2), F32),
        *[pltpu.VMEM((1, KB // 2, NQ), U32)] * NSLOT,
        pltpu.VMEM((16, 128), F32),
        pltpu.VMEM((16, 128), BF16),
        pltpu.VMEM((1, D), BF16),
        pltpu.SemaphoreType.DMA((15,)),
        pltpu.SemaphoreType.DMA((len(out_blocks),)),
    ]

    def fused(A_x, A_wq, A_wk, A_wv, A_wo, B_x, B_w_in, B_w_sp, B_b_sp, B_w_out, c, w_mod):
        del B_x
        out = pl.pallas_call(
            kernel,
            out_shape=jax.ShapeDtypeStruct((S, D), BF16),
            in_specs=[pl.BlockSpec(memory_space=pl.ANY)] * 11,
            out_specs=pl.BlockSpec(memory_space=pl.ANY),
            scratch_shapes=scratch,
            compiler_params=pltpu.CompilerParams(vmem_limit_bytes=120 * 1024 * 1024, flags=flags),
        )(A_x.reshape(S, D), A_wq, A_wk.T, A_wv.T, A_wo, B_w_in, B_w_sp, B_b_sp.reshape(16, 128), B_w_out,
          c, w_mod)
        return out.reshape(1, S, D)

    return fused


_fused = make(U=8)


@jax.jit
def pallas_adaLN_cond__grouped_kv_mqa__mixer_gmlp__prompt_kernel(
    A_x, A_wq, A_wk, A_wv, A_wo, B_x, B_w_in, B_w_sp, B_b_sp, B_w_out, c, w_mod,
):
    return _fused(A_x, A_wq, A_wk, A_wv, A_wo, B_x, B_w_in, B_w_sp, B_b_sp, B_w_out, c, w_mod)
```

```python
import bisect
import math

import jax
import jax.numpy as jnp
from jax import lax
import jax.experimental.pallas as pl
import jax.experimental.pallas.tpu as pltpu

F32 = jnp.float32
BF16 = jnp.bfloat16
U32 = jnp.uint32

S, D, H, DH, F, FH = 2048, 512, 32, 16, 1792, 896
NQ = 512
NT = NQ // 128
NJ = S // NQ
KB = 128
NKB = S // KB
EPS = 1e-5
QSCALE = DH ** -0.5 * math.log2(math.e)
SAFE_BOUND = 64.0
NSLOT = 4
NZ = 64

NT_DIMS = (((1,), (1,)), ((), ()))

STRASSEN = [
    ([((1, 0), 1), ((1, 1), 1)], [((0, 0), 1)], [((1, 0), 1), ((1, 1), -1)]),
    ([((1, 1), 1)], [((1, 0), 1), ((0, 0), -1)], [((0, 0), 1), ((1, 0), 1)]),
    ([((0, 0), 1), ((1, 1), 1)], [((0, 0), 1), ((1, 1), 1)], [((0, 0), 1), ((1, 1), 1)]),
    ([((0, 0), 1), ((0, 1), 1)], [((1, 1), 1)], [((0, 0), -1), ((0, 1), 1)]),
    ([((0, 1), 1), ((1, 1), -1)], [((1, 0), 1), ((1, 1), 1)], [((0, 0), 1)]),
    ([((0, 0), 1)], [((0, 1), 1), ((1, 1), -1)], [((0, 1), 1), ((1, 1), 1)]),
    ([((1, 0), 1), ((0, 0), -1)], [((0, 0), 1), ((0, 1), 1)], [((1, 1), 1)]),
]
CLASSIC = [([((i, k), 1)], [((k, j), 1)], [((i, j), 1)]) for j in range(2) for i in (1, 0) for k in range(2)]


def _lincomb(terms, get):
    acc = None
    for p, s in sorted(terms, key=lambda t: -t[1]):
        v = get(p)
        if acc is None:
            acc = v if s > 0 else -v
        else:
            acc = acc + v if s > 0 else acc - v
    return acc


def _touches_later(alg, i, p):
    return any(p == q for _, _, c in alg[i + 1:] for q, _ in c)


def _ln_cols(x):
    xc = x - jnp.mean(x, axis=0, keepdims=True)
    v = jnp.mean(xc * xc, axis=0, keepdims=True)
    return xc * lax.rsqrt(v + EPS)


def _gelu_of_half(hx):
    c0 = 2.0 * math.sqrt(2.0 / math.pi)
    c1 = c0 * 4.0 * 0.044715
    return hx + hx * jnp.tanh(hx * (c0 + c1 * (hx * hx)))


def _pack(x):
    return pltpu.bitcast(x.astype(BF16), U32)


def _pack2(x):
    return pltpu.pack_elementwise([x[0:8], x[8:16]], packed_dtype=BF16)


def _unpack(w):
    return pltpu.bitcast(w, BF16)


def _lanes(col, n):
    return jnp.concatenate([col] * (n // 128), axis=1)


def make(nv=(16, 16, 16, 32), U=8, skew=2, chains=2, phase=0.0, phases='B', flags=None, win_alg='s', sp_lv=2,
         out_blocks=((1024, 512), (1536, 512), (0, 512), (512, 256), (768, 128), (896, 128)), scopes=False, qstep=4, xwait=10, xlast=26, xcuts=(256, 512, 896), dorder=0, wchunk=1, opq=1, npair=1, wo_alg='c', wo_ord=(1, 0, 3, 2, 4, 5, 6), modfirst=True, fence_blocks=(4,), fence_products=((6, 5),), afence=0, bonly=False, eorder='n', wts=(31, 31, 33, 18), cpos=2, biters=None,
         win_ord=(1, 0, 2, 5, 6, 3, 4), out_ord=(5, 3, 2, 0, 6, 1, 4), in_ord=(5, 3, 2, 6, 0, 1, 4), back_at=(1, 1)):
    nvs = [nv[kb % len(nv)] for kb in range(NKB)]
    goff, moff = [0], [0]
    for n in nvs:
        goff.append(goff[-1] + n // 8)
        moff.append(moff[-1] + (KB - n) // 8)
    NG, NM = goff[-1], moff[-1]
    assert all(n % 16 == 0 for n in nvs) and NM % 2 == 0 and NG % 2 == 0 and NG <= NZ and U <= NZ
    qoff = [(m + 1) // 2 for m in moff]
    ysplit = (S, S // 2, 0)[npair]
    WIN = [STRASSEN[i] for i in win_ord] if win_alg == 's' else CLASSIC

    def kernel(x_hbm, wq_hbm, wkt_hbm, wvt_hbm, wo_hbm, win_hbm, wsp_hbm, bsp_hbm, wout_hbm, c_hbm, wmod_hbm,
               out_hbm,
               x_v, wq_v, wkt_v, wvt_v, wo_v, win_v, wsp_v, wout_v, wmod_v, out_v,
               zero_s, mod_s, wt_s, qt_s, qf0_s, qf1_s, kf_s, k_s, vt_s, kb_s, xt_s, ot_s, wot_s, wint_s, wina_s,
               woutt_s, wouta_s, h2a_s, h2b_s, z1_s, z2_s, g_s, y_s, wsum_s, macc_s, ge0_s, ge1_s, ge2_s, ge3_s, g1_s, p0_s, p1_s, p2_s, p3_s, b_s, bsp_v, c_v, fence_v,
               sem, osem):
        p_s = (p0_s, p1_s, p2_s, p3_s)
        qf_s = (qf0_s, qf1_s)
        h2_s = (h2a_s, h2b_s)
        ge_s = (ge0_s, ge1_s, ge2_s, ge3_s)
        import contextlib
        stack = contextlib.ExitStack()

        def mark(name):
            if scopes:
                stack.close()
                if name:
                    stack.enter_context(jax.named_scope(name))
        mark('A0_start')

        def cp(i, src, dst):
            return pltpu.make_async_copy(src, dst, sem.at[i])

        c_cp = cp(0, c_hbm, c_v)
        wmod_a_cp = cp(1, wmod_hbm.at[:, pl.ds(0, 2 * D)], wmod_v.at[:, pl.ds(0, 2 * D)])
        wq_cp = cp(2, wq_hbm, wq_v)
        wkt_cp = cp(3, wkt_hbm, wkt_v)
        wvt_cp = cp(4, wvt_hbm, wvt_v)
        x_cps = [cp(5 + i, x_hbm.at[pl.ds(lo, hi - lo)], x_v.at[pl.ds(lo, hi - lo)])
                 for i, (lo, hi) in enumerate(zip((0, *xcuts), (*xcuts, S)))]
        wmod_b_cp = cp(9, wmod_hbm.at[:, pl.ds(2 * D, 4 * D)], wmod_v.at[:, pl.ds(2 * D, 4 * D)])
        wo_cp = cp(10, wo_hbm, wo_v)
        win_cp = cp(11, win_hbm, win_v)
        bsp_cp = cp(12, bsp_hbm, bsp_v)
        wout_cp = cp(13, wout_hbm, wout_v)
        wsp_cp = cp(14, wsp_hbm, wsp_v)
        for d in ((c_cp, x_cps[0], wmod_a_cp, wkt_cp, wvt_cp, wq_cp, *x_cps[1:]),
                  (c_cp, wmod_a_cp, x_cps[0], wkt_cp, wvt_cp, wq_cp, *x_cps[1:]),
                  (c_cp, wkt_cp, wvt_cp, wq_cp, x_cps[0], wmod_a_cp, *x_cps[1:]))[dorder]:
            d.start()

        nf = len(fence_blocks) + len(fence_products) + (afence > 0)
        fences = [cp(15 + i, c_hbm, fence_v.at[i]) for i in range(nf)]
        for d in fences:
            d.start()

        def zinit(i, c):
            zero_s[i] = 0
            return c
        lax.fori_loop(0, NZ, zinit, 0)

        def transpose_into(dst, src, rows, cols, at=0):
            for i in range(cols // 128):
                dst[0, at + i * 64:at + (i + 1) * 64, :] = pltpu.bitcast(src[0:rows, i * 128:(i + 1) * 128].T, U32)

        def column_table(i, row):
            mod_s[i] = jnp.broadcast_to(row, (128, D)).T

        c_cp.wait()

        def mod_rows(lo, hi):
            cf = c_v[...].astype(F32)
            sc = jnp.broadcast_to(cf * jax.nn.sigmoid(cf), (16, D)).astype(BF16)
            return jnp.dot(sc, wmod_v[:, lo * D:hi * D], preferred_element_type=F32)[0:1]

        xn, kv = {}, {}
        bounds = [jnp.zeros((8, 128), F32), jnp.zeros((1, 128), F32), jnp.zeros((DH, 128), F32)]

        def a_norm(n):
            cols = slice(n * 128, (n + 1) * 128)
            xt = x_v[cols, :].T.astype(F32)
            xt_s[:, cols] = xt
            xn[n] = _ln_cols(xt)

        def a_proj(n, lo, hi):
            cols = slice(n * 128, (n + 1) * 128)
            if xn[n].dtype == F32:
                xn[n] = (xn[n] * mod_s[1] + mod_s[0]).astype(BF16)
            r = jnp.dot(_unpack(wt_s[zero_s[n], 8 * lo:8 * hi, :]), xn[n], preferred_element_type=F32)
            for i in range(max(lo, 2), hi):
                qf = r[(i - lo) * DH:(i - lo + 1) * DH] * QSCALE
                qt_s[(i - 2) * 8:(i - 1) * 8, cols] = _pack2(qf)
                bounds[0] = jnp.maximum(bounds[0], qf[0:8] * qf[0:8] + qf[8:16] * qf[8:16])
            if lo == 0:
                kv[n] = r[0:2 * DH]

        def a_keys(n):
            cols = slice(n * 128, (n + 1) * 128)
            r = kv.pop(n)
            kt = r[0:DH].astype(BF16).astype(F32)
            bounds[1] = jnp.maximum(bounds[1], jnp.sum(kt * kt, axis=0, keepdims=True))
            kf_s[cols, :] = kt.T
            bounds[2] = jnp.maximum(bounds[2], jnp.abs(r[DH:2 * DH]))
            vt_s[:, cols] = _pack(r[DH:2 * DH])
            for i in range(KB // 16):
                a1, a2 = (kf_s[pl.ds(n * KB + 16 * i + e, 8, stride=2), :] for e in range(2))
                if i < (KB - nvs[n]) // 16:
                    k_s[8 * (qoff[n] + i):8 * (qoff[n] + i + 1), :] = _pack(jnp.concatenate([a1, a2], axis=0))
                    continue
                g = goff[n] // 2 + i - (KB - nvs[n]) // 16
                for dd in range(8):
                    a11, a12, a21, a22 = (jnp.broadcast_to(a[:, e:e + 1], (8, 128))
                                          for a in (a1, a2) for e in (2 * dd, 2 * dd + 1))
                    for m, v in enumerate((a11 + a22, a21 + a22, a11, a22, a11 + a12, a21 - a11, a12 - a22)):
                        kb_s[g * 56 + m * 8 + dd] = v

        if not bonly:
          x_cps[0].wait()
        mark('A1_proj')
        if not bonly:
            for n in range(xcuts[0] // 128):
                a_norm(n)
            mark('A2_waitmod')
            wmod_a_cp.wait()
            mark('A3_mod')
            mod_a = mod_rows(0, 2)
            column_table(0, mod_a[0:1, 0:D])
            column_table(1, 1.0 + mod_a[0:1, D:2 * D])
            mark('A4_waitwq')
            wq_cp.wait()
            mark('A5_wq')
            transpose_into(wt_s, wq_v, D, D, at=DH)
            wkt_cp.wait()
            wvt_cp.wait()
            wt_s[0, 0:8, :] = _pack2(wkt_v[...].astype(F32))
            wt_s[0, 8:16, :] = pltpu.bitcast(wvt_v[...], U32)
            mark('A6_waitx1')
            x_cps[1].wait()
            mark('A7_first')
            ends = [c // 128 - 1 for c in xcuts[1:]] + [NKB - 1]
            for n in range(NKB):
                if n >= xcuts[0] // 128:
                    a_norm(n)
                cut = xwait if n < NKB - 2 else xlast
                if n + 1 in ends:
                    a_proj(n, 0, cut)
                elif n in ends:
                    a_proj(n, 0, 2)
                    if n < NKB - 1:
                        x_cps[2 + ends.index(n)].wait()
                    if n == ends[-2]:
                        for d in (wo_cp, wmod_b_cp, win_cp, bsp_cp, wout_cp, wsp_cp):
                            d.start()
                    a_proj(n - 1, cut, H + 2)
                    if n == NKB - 1 and afence > 2:
                        a_proj(n, 2, afence)
                    a_keys(n - 1)
                    a_keys(n)
                    if n == NKB - 1 and afence:
                        fences.pop().wait()
                    a_proj(n, max(afence, 2) if n == NKB - 1 else 2, H + 2)
                else:
                    a_proj(n, 0, H + 2)
                    a_keys(n)
        qmax, kmax, vmax = bounds

        safe = jnp.logical_and(
            jnp.max(jnp.sum(qmax, axis=0, keepdims=True)) * jnp.max(kmax) <= SAFE_BOUND * SAFE_BOUND,
            jnp.max(vmax) <= 2.0 ** 40)

        mark('B_att')
        def getq(h, j):
            if isinstance(h, int) and isinstance(j, int):
                return qt_s[h * 8:(h + 1) * 8, j * NQ:(j + 1) * NQ]
            return qt_s[pl.ds(pl.multiple_of(h * 8, 8), 8), pl.ds(pl.multiple_of(j * NQ, NQ), NQ)]

        def puto(h, j, val):
            if isinstance(h, int) and isinstance(j, int):
                ot_s[h * 8:(h + 1) * 8, j * NQ:(j + 1) * NQ] = _pack(val)
                return
            ot_s[pl.ds(pl.multiple_of(h * 8, 8), 8), pl.ds(pl.multiple_of(j * NQ, NQ), NQ)] = _pack(val)

        def query_table(slot, h, j):
            lo, hi = (pltpu.unpack_elementwise(getq(h, j), index=e, packed_dtype=BF16, unpacked_dtype=F32)
                      for e in range(2))
            for m in range(NT // 2):
                b11, b12 = lo[:, 256 * m:256 * m + 128], lo[:, 256 * m + 128:256 * m + 256]
                b21, b22 = hi[:, 256 * m:256 * m + 128], hi[:, 256 * m + 128:256 * m + 256]
                for i, v in enumerate((b11 + b22, b11, b12 - b22, b21 - b11, b22, b11 + b12, b21 + b22)):
                    qf_s[slot][0, 8 * i:8 * i + 8, m * 128:(m + 1) * 128] = v

        def pv_tile(t):
            u, kb = divmod(t, NKB)
            pb = _unpack(p_s[t % NSLOT][zero_s[t % NZ]])
            vb = _unpack(vt_s[:, pl.ds(pl.multiple_of(kb * KB + zero_s[u % NZ] * 128, 128), KB)])
            return jnp.dot(vb, pb, preferred_element_type=F32)

        def finish(h, j, acc, lsum):
            l = jnp.sum(lsum, axis=0, keepdims=True)
            r = pl.reciprocal(l, approx=True)
            puto(h, j, acc * (r * (2.0 - l * r)))

        def fast_body(it, carry):
            j = it // (H // U)
            h0 = (it % (H // U)) * U
            scores, pend, lsum, acc, done = {}, {}, {}, {}, {}
            items = [(g, o) for g in range(0, NG, 2) for o in range(4)]
            weights = [0]
            for _, o in items:
                weights.append(weights[-1] + wts[o])
            memo = {}

            def vpu_scores(u, g, o):
                zk = zero_s[u]
                zq = zero_s[g]

                def prod(i):
                    ks = [kb_s[(g // 2) * 56 + i * 8 + dd + zk] for dd in range(8)]
                    res = []
                    for m in range(2):
                        a = [None] * chains
                        for dd in range(8):
                            row = qf_s[u % 2][zq, 8 * i + dd:8 * i + dd + 1, m * 128:(m + 1) * 128]
                            pr = ks[dd] * jnp.broadcast_to(row, (8, 128))
                            a[dd % chains] = pr if dd < chains else a[dd % chains] + pr
                        while len(a) > 1:
                            a = [a[e] + a[e + 1] for e in range(0, len(a), 2)]
                        res.append(a[0])
                    return res

                def add(a, b):
                    return [x + y for x, y in zip(a, b)]

                def sub(a, b):
                    return [x - y for x, y in zip(a, b)]

                if o == 0:
                    memo[3], memo[5] = prod(2), prod(4)
                    return g, 1, add(memo[3], memo[5])
                if o == 1:
                    memo[2], memo[4] = prod(1), prod(3)
                    return g + 1, 0, add(memo[2], memo[4])
                if o == 2:
                    part = add(sub(memo.pop(4), memo.pop(5)), prod(6))
                    memo[1] = prod(0)
                    return g, 0, add(part, memo[1])
                return g + 1, 1, add(add(sub(memo.pop(3), memo.pop(2)), memo.pop(1)), prod(5))

            def emit(u, kb, r, n, s):
                p = jnp.exp2(s)
                lsum[u, n] = p if (u, n) not in lsum else lsum[u, n] + p
                t = u * NKB + kb
                if (t, r ^ 1, n) in pend:
                    o = pend.pop((t, r ^ 1, n))
                    p_s[t % NSLOT][0, 8 * (r // 2):8 * (r // 2) + 8, n * 128:(n + 1) * 128] = (
                        pltpu.pack_elementwise([p, o] if r % 2 == 0 else [o, p], packed_dtype=BF16))
                else:
                    pend[t, r, n] = p

            def do_items(u, upto):
                while done.get(u, 0) < upto:
                    g, n, ss = vpu_scores(u, *items[done.get(u, 0)])
                    done[u] = done.get(u, 0) + 1
                    kb = bisect.bisect_right(goff, g) - 1
                    for m, s in enumerate(ss):
                        emit(u, kb, (KB - nvs[kb]) // 8 + g - goff[kb], 2 * m + n, s)

            def soft(t):
                u, kb = divmod(t, NKB)
                s = scores.pop(t)
                for i in range(qoff[kb], qoff[kb + 1]):
                    ne = [(n, e) for n in range(NT) for e in range(2)]
                    for k, (n, e) in enumerate(ne if eorder == 'n' else sorted(ne, key=lambda x: x[1])):
                        r0 = 16 * (i - qoff[kb]) + 8 * e
                        kb2 = bisect.bisect_right(moff, 2 * i + e) - 1
                        emit(u, kb2, 2 * i + e - moff[kb2], n, s[r0:r0 + 8, n * 128:(n + 1) * 128])
                        if (k + 1) % (8 // cpos) == 0:
                            do_items(u, min(len(items), bisect.bisect_left(
                                weights, (i + (k + 1) / 8 + phase) / (NM // 2) * weights[-1] - 1e-9)))
                do_items(u, (goff[kb + 1] + 1) // 2 * 4)

            T = U * NKB
            prev = (it + NJ * H // U - 1) % (NJ * H // U)
            acc[-1], lsum[-1] = carry
            for t in range(T):
                u, kb = divmod(t, NKB)
                if kb == 0:
                    q = _unpack(getq(h0 + u, j))
                kk = k_s[pl.ds(pl.multiple_of(8 * qoff[kb] + zero_s[u] * 8, 8), 8 * (qoff[kb + 1] - qoff[kb])), :]
                scores[t] = jnp.dot(_unpack(kk), q, preferred_element_type=F32)
                if kb == qstep and u + 1 < U:
                    query_table((u + 1) % 2, h0 + u + 1, j)
                elif kb == qstep:
                    nxt = jnp.minimum(it + 1, NJ * H // U - 1)
                    query_table(0, (nxt % (H // U)) * U, nxt // (H // U))
                if t >= 1:
                    soft(t - 1)
                u, kb = divmod(t - skew, NKB)
                d = pv_tile(t - skew)
                acc[u] = d if kb == 0 else acc[u] + d
                if kb == NKB - 1 and u < 0:
                    finish((prev % (H // U)) * U + U - 1, prev // (H // U), acc[u], lsum[u])
                elif kb == NKB - 1:
                    finish(h0 + u, j, acc[u], jnp.concatenate([lsum[u, n] for n in range(NT)], axis=1))
            soft(T - 1)
            return acc[U - 1], jnp.concatenate([lsum[U - 1, n] for n in range(NT)], axis=1)

        def slow_body(it, carry):
            j = it // H
            h = it % H
            s = jnp.dot(kf_s[...].astype(BF16), _unpack(getq(h, j)), preferred_element_type=F32)
            p = jnp.exp2(s - jnp.max(s, axis=0, keepdims=True))
            l = jnp.sum(p, axis=0, keepdims=True)
            o = jnp.dot(_unpack(vt_s[...]), p.astype(BF16), preferred_element_type=F32)
            puto(h, j, o * (1.0 / l))
            return carry

        if 'B' in phases:
            @pl.when(safe)
            def _():
                query_table(0, 0, 0)
                for t in range(-skew, 0):
                    p_s[t % NSLOT][...] = jnp.zeros(p_s[0].shape, U32)
                acc, lsum = lax.fori_loop(0, biters or NJ * H // U, fast_body,
                                          (jnp.zeros((DH, NQ), F32), jnp.ones((8, NQ), F32)))
                for t in range(-skew, 0):
                    acc = acc + pv_tile(t)
                finish(H - 1, NJ - 1, acc, lsum)

            @pl.when(jnp.logical_not(safe))
            def _():
                lax.fori_loop(0, NJ * H, slow_body, 0)
        else:
            ot_s[...] = jnp.zeros(ot_s.shape, U32)

        if bonly:
            out_v[0:256, :] = _unpack(ot_s[0:128, 0:512])
            return
        mark('C0_prep')
        for d in (wo_cp, wmod_b_cp, win_cp, bsp_cp, wout_cp, wsp_cp):
            d.wait()
        transpose_into(wot_s, wo_v, D, D)

        def mod_row(i):
            return mod_rows(i, i + 1)

        column_table(2, mod_row(2))
        b_s[...] = bsp_v[...].astype(F32)

        mark('C1_wo')
        transposed = set()

        def win_block(p, sub):
            cols = slice(p[1] * 256, (p[1] + 1) * 256)
            for i in range(sub.start // 128, (sub.stop + 127) // 128):
                if (p, i) not in transposed:
                    transposed.add((p, i))
                    rows = slice(p[0] * FH + i * 128, p[0] * FH + (i + 1) * 128)
                    wint_s[rows, cols] = win_v[cols, rows].T.astype(F32)
            return wint_s[p[0] * FH + sub.start:p[0] * FH + sub.stop, cols]

        def c_norm(j, a):
            cols = slice(j * NQ, (j + 1) * NQ)
            x1 = xt_s[:, cols] + _lanes(mod_s[2], NQ) * a
            xt_s[:, cols] = x1
            h2_s[j // 2][0, :, (j % 2) * NQ:(j % 2 + 1) * NQ] = _ln_cols(x1) * _lanes(mod_s[4], NQ) + _lanes(mod_s[3], NQ)

        def halved_tables():
            column_table(3, 0.5 * mod_row(3))
            column_table(4, 0.5 + 0.5 * mod_row(4))

        if modfirst:
            halved_tables()
        if wo_alg == 'c':
            for j in range(NJ):
                c_norm(j, jnp.dot(_unpack(wot_s[zero_s[j]]), _unpack(ot_s[:, j * NQ:(j + 1) * NQ]),
                                  preferred_element_type=F32))
        else:
            WO = [STRASSEN[i] for i in wo_ord]

            def operand(terms, get):
                if len(terms) == 1:
                    return _unpack(get(terms[0][0]))
                return _lincomb(terms, lambda p: _unpack(get(p)).astype(F32)).astype(BF16)

            aops = {}
            for pair in range(NJ // 2):
                acc = {}
                for i, (at, bt, ct) in enumerate(WO):
                    if pair == 0:
                        aops[i] = operand(at, lambda p: wot_s[zero_s[i], p[0] * 128:(p[0] + 1) * 128,
                                                              p[1] * 256:(p[1] + 1) * 256])
                    b = operand(bt, lambda p: ot_s[p[0] * 128:(p[0] + 1) * 128,
                                                   (2 * pair + p[1]) * NQ:(2 * pair + p[1] + 1) * NQ])
                    m = jnp.dot(aops[i], b, preferred_element_type=F32)
                    if pair == 0 and i == 1 and not modfirst:
                        halved_tables()
                    for p, sg in ct:
                        acc[p] = (m if sg > 0 else -m) if p not in acc else (acc[p] + m if sg > 0 else acc[p] - m)
                    for n in range(2):
                        if (0, n) in acc and (1, n) in acc and not any(_touches_later(WO, i, (r, n)) for r in range(2)):
                            c_norm(2 * pair + n, jnp.concatenate([acc.pop((0, n)), acc.pop((1, n))], axis=0))

        mark('C2_win')
        rc = FH // wchunk
        for pair in range(NJ // 2):
            bops, sums = {}, {}
            for ch in range(wchunk):
                rows = slice(ch * rc, (ch + 1) * rc)
                seen = set()
                for i, (at, bt, ct) in enumerate(WIN):
                    if pair == 0:
                        wina_s[i, ch * rc // 2:(ch + 1) * rc // 2, :] = _pack(_lincomb(at, lambda p: win_block(p, rows)))
                    if ch == 0:
                        bops[i] = _lincomb(bt, lambda p: h2_s[pair][zero_s[i] if opq & 4 else 0, p[0] * 256:(p[0] + 1) * 256,
                                                                    p[1] * NQ:(p[1] + 1) * NQ]).astype(BF16)
                    m = jnp.dot(_unpack(wina_s[i, ch * rc // 2:(ch + 1) * rc // 2, :]), bops[i],
                                preferred_element_type=F32)
                    for p, sg in ct:
                        dst = z2_s if p[0] else z1_s
                        cols = slice((2 * pair + p[1]) * NQ, (2 * pair + p[1] + 1) * NQ)
                        if p in seen:
                            val = dst[rows, cols] + m if sg > 0 else dst[rows, cols] - m
                        else:
                            seen.add(p)
                            val = m if sg > 0 else -m
                        if _touches_later(WIN, i, p):
                            dst[rows, cols] = val
                            continue
                        val = _gelu_of_half(val)
                        if p[0] and opq & 1:
                            ge_s[2 * pair + p[1]][0, rows, :] = val
                            part = jnp.sum(val.reshape(rc // 8, 8, NQ), axis=0)
                            sums[p[1]] = part if ch == 0 else sums[p[1]] + part
                        elif opq & 2 and not p[0]:
                            g1_s[0, rows, cols] = val
                        else:
                            dst[rows, cols] = val
            for n in range(2):
                cols = slice((2 * pair + n) * NQ, (2 * pair + n + 1) * NQ)
                if opq & 1:
                    xc = ge_s[2 * pair + n][zero_s[n]] - jnp.sum(sums[n], axis=0, keepdims=True) * (1.0 / FH)
                    z2_s[:, cols] = xc * lax.rsqrt(jnp.mean(xc * xc, axis=0, keepdims=True) + EPS)
                else:
                    z2_s[:, cols] = _ln_cols(z2_s[:, cols])

        mark('D')
        def out_cp(i):
            rows = pl.ds(*out_blocks[i])
            return pltpu.make_async_copy(out_v.at[rows], out_hbm.at[rows], osem.at[i])

        def d_store(i, y):
            if i in fence_blocks:
                fences.pop().wait()
            cols = slice(out_blocks[i][0], out_blocks[i][0] + out_blocks[i][1])
            out_v[cols, :] = (xt_s[:, cols] + _lanes(mod_s[5], out_blocks[i][1]) * y).astype(BF16).T
            out_cp(i).start()

        KH = 384

        def d_prepare():
            transpose_into(woutt_s, wout_v, FH, D)
            column_table(5, mod_row(5))
            if npair:
                for i, (at, _, _) in enumerate(STRASSEN):
                    wouta_s[i] = _pack(_lincomb(at, lambda p: _unpack(
                        woutt_s[zero_s[i], p[0] * 128:(p[0] + 1) * 128, p[1] * KH:(p[1] + 1) * KH]).astype(F32)))

        def d_back(i):
            cols = slice(out_blocks[i][0], out_blocks[i][0] + out_blocks[i][1])
            d_store(i, jnp.dot(_unpack(woutt_s[zero_s[i]]), gety(slice(0, FH), cols), preferred_element_type=F32))

        def gety(rows, cols):
            if cols.start >= ysplit:
                return g_s[rows, cols].astype(BF16)
            return _unpack(y_s[rows.start // 2:rows.stop // 2, cols])

        def d_back_pair(i, lo, hi, acc):
            cb = [slice(o, o + w) for o, w in out_blocks[i:i + 2]]
            for k in range(lo, hi):
                _, bt, ct = STRASSEN[k]
                b = _lincomb(bt, lambda p: g_s[p[0] * KH:(p[0] + 1) * KH, cb[p[1]]]).astype(BF16)
                m = jnp.dot(_unpack(wouta_s[k]), b, preferred_element_type=F32)
                for p, sg in ct:
                    acc[p] = (m if sg > 0 else -m) if p not in acc else (acc[p] + m if sg > 0 else acc[p] - m)
                for n in range(2):
                    if (0, n) in acc and not any(_touches_later(STRASSEN, k, (r, n)) for r in range(2)):
                        rest = jnp.dot(_unpack(woutt_s[zero_s[i + n], :, 2 * KH:]), gety(slice(2 * KH, FH), cb[n]),
                                       preferred_element_type=F32)
                        d_store(i + n, jnp.concatenate([acc.pop((0, n)), acc.pop((1, n))], axis=0) + rest)

        mb, kb_ = FH // 4, S // 4

        def gate(blk, val):
            rows = slice(blk[0] * mb, (blk[0] + 1) * mb)
            cols = slice(blk[1] * kb_, (blk[1] + 1) * kb_)
            bias = jnp.concatenate([b_s[i:i + 1, :] for i in range(4 * blk[1], 4 * blk[1] + 4)], axis=1)
            y = z1_s[rows, cols] * (val + bias)
            if cols.start >= ysplit:
                g_s[rows, cols] = y
            else:
                y_s[blk[0] * mb // 2:(blk[0] + 1) * mb // 2, cols] = _pack(y)

        def getz(p):
            return z2_s[p[0] * mb:(p[0] + 1) * mb, p[1] * kb_:(p[1] + 1) * kb_]

        def getw(p):
            return wsp_v[p[1] * kb_:(p[1] + 1) * kb_, p[0] * kb_:(p[0] + 1) * kb_]

        outer = [STRASSEN[i] for i in out_ord] if sp_lv >= 1 else CLASSIC
        inner = [STRASSEN[i] for i in in_ord] if sp_lv >= 2 else CLASSIC
        seen = set()
        nback, oacc = 0, {}
        for oi, (a1, b1, c1) in enumerate(outer):
            if len(b1) > 1:
                for r in range(2):
                    for cc in range(2):
                        wsum_s[oi % 2, r * kb_:(r + 1) * kb_, cc * kb_:(cc + 1) * kb_] = _lincomb(
                            b1, lambda p: getw((2 * p[0] + cc, 2 * p[1] + r)).astype(F32))
            seen2 = set()
            for ii, (a2, b2, c2) in enumerate(inner):
                a = _lincomb([((2 * p1[0] + p2[0], 2 * p1[1] + p2[1]), s1 * s2) for p1, s1 in a1 for p2, s2 in a2],
                             getz).astype(BF16)
                if len(b1) > 1:
                    b = _lincomb(b2, lambda p: wsum_s[oi % 2, p[1] * kb_:(p[1] + 1) * kb_,
                                                      p[0] * kb_:(p[0] + 1) * kb_]).astype(BF16)
                else:
                    p1 = b1[0][0]
                    if len(b2) > 1:
                        b = _lincomb(b2, lambda p: getw((2 * p1[0] + p[0], 2 * p1[1] + p[1])).astype(F32)).astype(BF16)
                    else:
                        b = getw((2 * p1[0] + b2[0][0][0], 2 * p1[1] + b2[0][0][1]))
                m = lax.dot_general(a, b, NT_DIMS, preferred_element_type=F32)
                for p, sg in c2:
                    sl = (slice(p[0] * mb, (p[0] + 1) * mb), slice(p[1] * kb_, (p[1] + 1) * kb_))
                    if p in seen2:
                        val = macc_s[sl] + m if sg > 0 else macc_s[sl] - m
                    else:
                        seen2.add(p)
                        val = m if sg > 0 else -m
                    if _touches_later(inner, ii, p):
                        macc_s[sl] = val
                        continue
                    for p1, s1 in c1:
                        blk = (2 * p1[0] + p[0], 2 * p1[1] + p[1])
                        gl = (slice(blk[0] * mb, (blk[0] + 1) * mb), slice(blk[1] * kb_, (blk[1] + 1) * kb_))
                        if blk in seen:
                            tot = g_s[gl] + val if s1 > 0 else g_s[gl] - val
                        else:
                            seen.add(blk)
                            tot = val if s1 > 0 else -val
                        if _touches_later(outer, oi, p1):
                            g_s[gl] = tot
                        else:
                            gate(blk, tot)
                half = out_blocks[0][0] // (S // 2)
                half_done = not any(q[1] == half for _, _, c in outer[oi:] for q, _ in c)
                if half_done and nback < 2 and ii == back_at[nback]:
                    if nback == 0:
                        d_prepare()
                    if npair:
                        d_back_pair(0, *((0, 4), (4, 7))[nback], oacc)
                    else:
                        d_back(nback)
                    nback += 1
                if (oi, ii) in fence_products:
                    fences.pop().wait()
        if npair == 2:
            d_back_pair(2, 0, 7, {})
            nback += 2
        while nback < len(out_blocks):
            d_back(nback)
            nback += 1
        mark('E_tail')
        for i in range(len(out_blocks)):
            out_cp(i).wait()
        mark(None)

    scratch = [
        pltpu.VMEM((S, D), BF16),
        pltpu.VMEM((D, D), BF16),
        pltpu.VMEM((DH, D), BF16),
        pltpu.VMEM((DH, D), BF16),
        pltpu.VMEM((D, D), BF16),
        pltpu.VMEM((D, F), BF16),
        pltpu.VMEM((S, S), BF16),
        pltpu.VMEM((FH, D), BF16),
        pltpu.VMEM((D, 6 * D), BF16),
        pltpu.VMEM((S, D), BF16),
        pltpu.SMEM((NZ,), jnp.int32),
        pltpu.VMEM((6, D, 128), F32),
        pltpu.VMEM((1, D // 2 + DH, D), U32),
        pltpu.VMEM((D // 2, S), U32),
        *[pltpu.VMEM((1, 64, NQ // 2), F32)] * 2,
        pltpu.VMEM((S, DH), F32),
        pltpu.VMEM((S // 2, DH), U32),
        pltpu.VMEM((DH // 2, S), U32),
        pltpu.VMEM((max(NG, 2) // 2 * 56, 8, 128), F32),
        pltpu.VMEM((D, S), F32),
        pltpu.VMEM((D // 2, S), U32),
        pltpu.VMEM((1, D // 2, D), U32),
        pltpu.VMEM((F, D), F32),
        pltpu.VMEM((len(WIN), FH // 2, 256), U32),
        pltpu.VMEM((1, D // 2, FH), U32),
        pltpu.VMEM((7, D // 4, 384), U32),
        *[pltpu.VMEM((1, D, S // 2), F32)] * 2,
        pltpu.VMEM((FH, S), F32),
        pltpu.VMEM((FH, S), F32),
        pltpu.VMEM((FH, S), F32),
        pltpu.VMEM((FH // 2, S), U32),
        pltpu.VMEM((2, S // 2, S // 2), F32),
        pltpu.VMEM((FH // 2, S // 2), F32),
        *[pltpu.VMEM((1, FH, NQ) if opq & 1 else (1, 8, 512), F32)] * 4,
        pltpu.VMEM((1, FH, S) if opq & 2 else (1, 8, 512), F32),
        *[pltpu.VMEM((1, KB // 2, NQ), U32)] * NSLOT,
        pltpu.VMEM((16, 128), F32),
        pltpu.VMEM((16, 128), BF16),
        pltpu.VMEM((1, D), BF16),
        pltpu.VMEM((8, 1, D), BF16),
        pltpu.SemaphoreType.DMA((23,)),
        pltpu.SemaphoreType.DMA((len(out_blocks),)),
    ]

    def fused(A_x, A_wq, A_wk, A_wv, A_wo, B_x, B_w_in, B_w_sp, B_b_sp, B_w_out, c, w_mod):
        del B_x
        out = pl.pallas_call(
            kernel,
            out_shape=jax.ShapeDtypeStruct((S, D), BF16),
            in_specs=[pl.BlockSpec(memory_space=pl.ANY)] * 11,
            out_specs=pl.BlockSpec(memory_space=pl.ANY),
            scratch_shapes=scratch,
            compiler_params=pltpu.CompilerParams(vmem_limit_bytes=120 * 1024 * 1024, flags=flags),
        )(A_x.reshape(S, D), A_wq, A_wk.T, A_wv.T, A_wo, B_w_in, B_w_sp, B_b_sp.reshape(16, 128), B_w_out,
          c, w_mod)
        return out.reshape(1, S, D)

    return fused


_fused = make(U=8, chains=4)


@jax.jit
def pallas_adaLN_cond__grouped_kv_mqa__mixer_gmlp__prompt_kernel(
    A_x, A_wq, A_wk, A_wv, A_wo, B_x, B_w_in, B_w_sp, B_b_sp, B_w_out, c, w_mod,
):
    return _fused(A_x, A_wq, A_wk, A_wv, A_wo, B_x, B_w_in, B_w_sp, B_b_sp, B_w_out, c, w_mod)
```

```python
import bisect
import math

import jax
import jax.numpy as jnp
from jax import lax
import jax.experimental.pallas as pl
import jax.experimental.pallas.tpu as pltpu

F32 = jnp.float32
BF16 = jnp.bfloat16
U32 = jnp.uint32

S, D, H, DH, F, FH = 2048, 512, 32, 16, 1792, 896
EPS = 1e-5
QSCALE = DH ** -0.5 * math.log2(math.e)

NQ = 512
NT = NQ // 128
NJ = S // NQ
KB = 128
NKB = S // KB
UNITS = 8
NIT = NJ * H // UNITS
SKEW = 2
NSLOT = 4
VPU_KEYS = (16, 16, 16, 32) * (NKB // 4)
SAFE_BOUND = 64.0
NZERO = 64

MXU_OFF = [sum(KB - n for n in VPU_KEYS[:t]) // 16 for t in range(NKB + 1)]
VPU_OFF = [sum(VPU_KEYS[:t]) // 16 for t in range(NKB + 1)]

X_CUTS = (0, 256, 512, 896, S)
OUT_BLOCKS = ((1024, 512), (1536, 512), (0, 512), (512, 256), (768, 128), (896, 128))
KH = 384

NT_DIMS = (((1,), (1,)), ((), ()))

M1 = ([((0, 0), 1), ((1, 1), 1)], [((0, 0), 1), ((1, 1), 1)], [((0, 0), 1), ((1, 1), 1)])
M2 = ([((1, 0), 1), ((1, 1), 1)], [((0, 0), 1)], [((1, 0), 1), ((1, 1), -1)])
M3 = ([((0, 0), 1)], [((0, 1), 1), ((1, 1), -1)], [((0, 1), 1), ((1, 1), 1)])
M4 = ([((1, 1), 1)], [((1, 0), 1), ((0, 0), -1)], [((0, 0), 1), ((1, 0), 1)])
M5 = ([((0, 0), 1), ((0, 1), 1)], [((1, 1), 1)], [((0, 0), -1), ((0, 1), 1)])
M6 = ([((1, 0), 1), ((0, 0), -1)], [((0, 0), 1), ((0, 1), 1)], [((1, 1), 1)])
M7 = ([((0, 1), 1), ((1, 1), -1)], [((1, 0), 1), ((1, 1), 1)], [((0, 0), 1)])
WIN_ORDER = (M4, M2, M1, M3, M5, M6, M7)
SP_OUTER = (M3, M5, M1, M2, M6, M4, M7)
SP_INNER = (M3, M5, M1, M6, M2, M4, M7)
OUT_ORDER = (M2, M4, M1, M5, M7, M3, M6)


def _lincomb(terms, get):
    acc = None
    for p, sign in sorted(terms, key=lambda t: -t[1]):
        acc = _accumulate(acc, get(p), sign)
    return acc


def _accumulate(acc, v, sign):
    if acc is None:
        return v if sign > 0 else -v
    return acc + v if sign > 0 else acc - v


def _nest(outer, inner):
    return [((2 * p[0] + q[0], 2 * p[1] + q[1]), a * b) for p, a in outer for q, b in inner]


def _pending(products, i, block):
    return any(block == p for _, _, c in products[i + 1:] for p, _ in c)


def _layernorm(x):
    xc = x - jnp.mean(x, axis=0, keepdims=True)
    return xc * lax.rsqrt(jnp.mean(xc * xc, axis=0, keepdims=True) + EPS)


def _gelu_of_half(hx):
    c0 = 2.0 * math.sqrt(2.0 / math.pi)
    c1 = c0 * 4.0 * 0.044715
    return hx + hx * jnp.tanh(hx * (c0 + c1 * (hx * hx)))


def _pack(x):
    return pltpu.bitcast(x.astype(BF16), U32)


def _unpack(w):
    return pltpu.bitcast(w, BF16)


def _lanes(col, n):
    return jnp.concatenate([col] * (n // 128), axis=1)


def _span(i, size):
    return slice(i * size, (i + 1) * size)


def _kernel(x_hbm, wq_hbm, wkt_hbm, wvt_hbm, wo_hbm, win_hbm, wsp_hbm, bsp_hbm, wout_hbm, c_hbm, wmod_hbm,
            out_hbm,
            x_v, wq_v, wkt_v, wvt_v, wo_v, win_v, wsp_v, wout_v, wmod_v, out_v,
            mod_s, wt_s, qt_s, qtab0_s, qtab1_s, kf_s, k_s, vt_s, ktab_s, p0_s, p1_s, p2_s, p3_s, xt_s, ot_s,
            wot_s, wint_s, woutt_s, wouta_s, h2_s, z1_s, z2_s, ge0_s, ge1_s, ge2_s, ge3_s,
            g_s, y_s, wsum_s, macc_s, b_s, bsp_v, c_v, fence_v,
            zero_s, sem, osem):
    p_s = (p0_s, p1_s, p2_s, p3_s)
    qtab_s = (qtab0_s, qtab1_s)
    ge_s = (ge0_s, ge1_s, ge2_s, ge3_s)

    copies = []

    def copy(src, dst):
        copies.append(pltpu.make_async_copy(src, dst, sem.at[len(copies)]))
        return copies[-1]

    c_cp = copy(c_hbm, c_v)
    x_cps = [copy(x_hbm.at[pl.ds(lo, hi - lo)], x_v.at[pl.ds(lo, hi - lo)]) for lo, hi in zip(X_CUTS, X_CUTS[1:])]
    wmod_a_cp = copy(wmod_hbm.at[:, pl.ds(0, 2 * D)], wmod_v.at[:, pl.ds(0, 2 * D)])
    wkt_cp = copy(wkt_hbm, wkt_v)
    wvt_cp = copy(wvt_hbm, wvt_v)
    wq_cp = copy(wq_hbm, wq_v)
    late_cps = [copy(wo_hbm, wo_v),
                copy(wmod_hbm.at[:, pl.ds(2 * D, 4 * D)], wmod_v.at[:, pl.ds(2 * D, 4 * D)]),
                copy(win_hbm, win_v), copy(bsp_hbm, bsp_v), copy(wout_hbm, wout_v), copy(wsp_hbm, wsp_v)]
    fences = [copy(c_hbm, fence_v.at[i]) for i in range(2)]
    for cp in (c_cp, x_cps[0], wmod_a_cp, wkt_cp, wvt_cp, wq_cp, *x_cps[1:], *fences):
        cp.start()

    def init_zero(i, carry):
        zero_s[i] = 0
        return carry
    lax.fori_loop(0, NZERO, init_zero, 0)

    def transpose_into(dst, src, at=0):
        for i in range(src.shape[1] // 128):
            dst[0, at + i * 64:at + (i + 1) * 64, :] = pltpu.bitcast(src[:, _span(i, 128)].T, U32)

    def mod_rows(lo, hi):
        cf = c_v[...].astype(F32)
        sc = jnp.broadcast_to(cf * jax.nn.sigmoid(cf), (16, D)).astype(BF16)
        return jnp.dot(sc, wmod_v[:, lo * D:hi * D], preferred_element_type=F32)[0:1]

    def column_table(i, row):
        mod_s[i] = jnp.broadcast_to(row, (128, D)).T

    normed, kv = {}, {}
    bounds = [jnp.zeros((8, 128), F32), jnp.zeros((1, 128), F32), jnp.zeros((DH, 128), F32)]

    def a_norm(n):
        xt = x_v[_span(n, 128), :].T.astype(F32)
        xt_s[:, _span(n, 128)] = xt
        normed[n] = _layernorm(xt)

    def a_project(n, lo, hi):
        if normed[n].dtype == F32:
            normed[n] = (normed[n] * mod_s[1] + mod_s[0]).astype(BF16)
        r = jnp.dot(_unpack(wt_s[zero_s[n], 8 * lo:8 * hi, :]), normed[n], preferred_element_type=F32)
        for i in range(max(lo, 2), hi):
            q = r[_span(i - lo, DH)] * QSCALE
            qt_s[_span(i - 2, 8), _span(n, 128)] = _pack(q)
            bounds[0] = jnp.maximum(bounds[0], q[0:8] * q[0:8] + q[8:16] * q[8:16])
        if lo == 0:
            kv[n] = r[0:2 * DH]

    def a_keys(n):
        r = kv.pop(n)
        kt = r[0:DH].astype(BF16).astype(F32)
        bounds[1] = jnp.maximum(bounds[1], jnp.sum(kt * kt, axis=0, keepdims=True))
        kf_s[_span(n, 128), :] = kt.T
        bounds[2] = jnp.maximum(bounds[2], jnp.abs(r[DH:2 * DH]))
        vt_s[:, _span(n, 128)] = _pack(r[DH:2 * DH])
        num_mxu = MXU_OFF[n + 1] - MXU_OFF[n]
        for i in range(KB // 16):
            k1, k2 = (kf_s[_span(16 * n + 2 * i + e, 8), :] for e in range(2))
            if i < num_mxu:
                k_s[_span(MXU_OFF[n] + i, 8), :] = _pack(jnp.concatenate([k1, k2], axis=0))
                continue
            for d in range(8):
                a11, a12, a21, a22 = (jnp.broadcast_to(k[:, e:e + 1], (8, 128)) for k in (k1, k2) for e in (d, d + 8))
                for m, v in enumerate((a11 + a22, a21 + a22, a11, a22, a11 + a12, a21 - a11, a12 - a22)):
                    ktab_s[(VPU_OFF[n] + i - num_mxu) * 56 + m * 8 + d] = v

    c_cp.wait()
    x_cps[0].wait()
    for n in range(X_CUTS[1] // 128):
        a_norm(n)
    wmod_a_cp.wait()
    mod_a = mod_rows(0, 2)
    column_table(0, mod_a[:, 0:D])
    column_table(1, 1.0 + mod_a[:, D:2 * D])
    wq_cp.wait()
    transpose_into(wt_s, wq_v, at=DH)
    wkt_cp.wait()
    wvt_cp.wait()
    wt_s[0, 0:8, :] = pltpu.bitcast(wkt_v[...], U32)
    wt_s[0, 8:16, :] = pltpu.bitcast(wvt_v[...], U32)
    x_cps[1].wait()
    last_tiles = [cut // 128 - 1 for cut in X_CUTS[2:]]
    for n in range(NKB):
        if n >= X_CUTS[1] // 128:
            a_norm(n)
        split = 10 if n < NKB - 2 else 26
        if n + 1 in last_tiles:
            a_project(n, 0, split)
        elif n in last_tiles:
            a_project(n, 0, 2)
            if n < NKB - 1:
                x_cps[2 + last_tiles.index(n)].wait()
            if n == last_tiles[-2]:
                for cp in late_cps:
                    cp.start()
            a_project(n - 1, split, H + 2)
            a_keys(n - 1)
            a_keys(n)
            a_project(n, 2, H + 2)
        else:
            a_project(n, 0, H + 2)
            a_keys(n)

    q2, k2, vmax = jnp.max(jnp.sum(bounds[0], axis=0, keepdims=True)), jnp.max(bounds[1]), jnp.max(bounds[2])
    safe = jnp.logical_and(q2 * k2 <= SAFE_BOUND * SAFE_BOUND, vmax <= 2.0 ** 40)

    def unit_index(h, j):
        if isinstance(h, int):
            return _span(h, 8), _span(j, NQ)
        return pl.ds(pl.multiple_of(h * 8, 8), 8), pl.ds(pl.multiple_of(j * NQ, NQ), NQ)

    def first_unit(it):
        return (it % (H // UNITS)) * UNITS, it // (H // UNITS)

    def query_table(slot, h, j):
        q = _unpack(qt_s[unit_index(h, j)]).astype(F32)
        for m in range(NT // 2):
            b11, b12, b21, b22 = (q[_span(r, 8), _span(2 * m + e, 128)] for r in range(2) for e in range(2))
            for i, v in enumerate((b11 + b22, b11, b12 - b22, b21 - b11, b22, b11 + b12, b21 + b22)):
                qtab_s[slot][0, _span(i, 8), _span(m, 128)] = v

    def pv_tile(t):
        u, kb = divmod(t, NKB)
        p = p_s[t % NSLOT][pl.ds(pl.multiple_of(zero_s[t % NZERO] * 8, 8), KB // 2), :]
        v = vt_s[:, pl.ds(pl.multiple_of(kb * KB + zero_s[u % NZERO] * 128, 128), KB)]
        return jnp.dot(_unpack(v), _unpack(p), preferred_element_type=F32)

    def finish(h, j, acc, sums):
        l = jnp.sum(sums, axis=0, keepdims=True)
        r = pl.reciprocal(l, approx=True)
        ot_s[unit_index(h, j)] = _pack(acc * (r * (2.0 - l * r)))

    def unshifted_body(it, carry):
        h0, j = first_unit(it)
        scores, halves, sums, acc, issued, products = {}, {}, {}, {}, {}, {}
        quarters = [(g, o) for g in range(VPU_OFF[-1]) for o in range(4)]
        work = [0]
        for _, o in quarters:
            work.append(work[-1] + (31, 31, 33, 18)[o])

        def valu_scores(u, g, o):
            zk, zq = zero_s[u], zero_s[2 * g]

            def product(i):
                keys = [ktab_s[g * 56 + i * 8 + d + zk] for d in range(8)]
                res = []
                for m in range(2):
                    t = [keys[d] * qtab_s[u % 2][zq, _span(8 * i + d, 1), _span(m, 128)] for d in range(8)]
                    t = [t[d] + t[d + 4] for d in range(4)]
                    res.append((t[0] + t[1]) + (t[2] + t[3]))
                return res

            def add(a, b):
                return [x + y for x, y in zip(a, b)]

            def sub(a, b):
                return [x - y for x, y in zip(a, b)]

            if o == 0:
                products[3], products[5] = product(2), product(4)
                return 0, 1, add(products[3], products[5])
            if o == 1:
                products[2], products[4] = product(1), product(3)
                return 1, 0, add(products[2], products[4])
            if o == 2:
                part = add(sub(products.pop(4), products.pop(5)), product(6))
                products[1] = product(0)
                return 0, 0, add(part, products[1])
            return 1, 1, add(add(sub(products.pop(3), products.pop(2)), products.pop(1)), product(5))

        def emit(t, group, half, n, s):
            u = t // NKB
            p = jnp.exp2(s)
            sums[u, n] = p if (u, n) not in sums else sums[u, n] + p
            if (t, group, n) not in halves:
                halves[t, group, n] = p
                return
            other = halves.pop((t, group, n))
            p_s[t % NSLOT][_span(group, 8), _span(n, 128)] = _pack(
                jnp.concatenate([other, p] if half else [p, other], axis=0))

        def issue_valu(u, upto):
            while issued.get(u, 0) < upto:
                g, o = quarters[issued.get(u, 0)]
                issued[u] = issued.get(u, 0) + 1
                kb = bisect.bisect_right(VPU_OFF, g) - 1
                half, n, res = valu_scores(u, g, o)
                for m, s in enumerate(res):
                    emit(u * NKB + kb, MXU_OFF[kb + 1] - MXU_OFF[kb] + g - VPU_OFF[kb], half, 2 * m + n, s)

        def exponentiate(t):
            u, kb = divmod(t, NKB)
            s = scores.pop(t)
            for i in range(MXU_OFF[kb + 1] - MXU_OFF[kb]):
                for n in range(NT):
                    for e in range(2):
                        emit(t, i, e, n, s[_span(2 * i + e, 8), _span(n, 128)])
                    if n % 2:
                        elapsed = (MXU_OFF[kb] + i + (n + 1) / NT) / MXU_OFF[-1]
                        issue_valu(u, min(len(quarters), bisect.bisect_left(work, elapsed * work[-1] - 1e-9)))
            issue_valu(u, 4 * VPU_OFF[kb + 1])

        def all_sums(u):
            return jnp.concatenate([sums[u, n] for n in range(NT)], axis=1)

        acc[-1], last_sums = carry
        for t in range(UNITS * NKB):
            u, kb = divmod(t, NKB)
            if kb == 0:
                q = _unpack(qt_s[unit_index(h0 + u, j)])
            k = k_s[pl.ds(pl.multiple_of(8 * MXU_OFF[kb] + zero_s[u] * 8, 8), 8 * (MXU_OFF[kb + 1] - MXU_OFF[kb])), :]
            scores[t] = jnp.dot(_unpack(k), q, preferred_element_type=F32)
            if kb == 4 and u + 1 < UNITS:
                query_table((u + 1) % 2, h0 + u + 1, j)
            elif kb == 4:
                query_table(0, *first_unit(jnp.minimum(it + 1, NIT - 1)))
            if t >= 1:
                exponentiate(t - 1)
            u, kb = divmod(t - SKEW, NKB)
            d = pv_tile(t - SKEW)
            acc[u] = d if kb == 0 else acc[u] + d
            if kb == NKB - 1 and u < 0:
                h_prev, j_prev = first_unit((it + NIT - 1) % NIT)
                finish(h_prev + UNITS - 1, j_prev, acc[u], last_sums)
            elif kb == NKB - 1:
                finish(h0 + u, j, acc[u], all_sums(u))
        exponentiate(UNITS * NKB - 1)
        return acc[UNITS - 1], all_sums(UNITS - 1)

    def shifted_body(it, carry):
        index = unit_index(it % H, it // H)
        s = jnp.dot(kf_s[...].astype(BF16), _unpack(qt_s[index]), preferred_element_type=F32)
        p = jnp.exp2(s - jnp.max(s, axis=0, keepdims=True))
        o = jnp.dot(_unpack(vt_s[...]), p.astype(BF16), preferred_element_type=F32)
        ot_s[index] = _pack(o * (1.0 / jnp.sum(p, axis=0, keepdims=True)))
        return carry

    @pl.when(safe)
    def _():
        query_table(0, 0, 0)
        for t in range(-SKEW, 0):
            p_s[t % NSLOT][...] = jnp.zeros(p_s[0].shape, U32)
        acc, sums = lax.fori_loop(0, NIT, unshifted_body, (jnp.zeros((DH, NQ), F32), jnp.ones((8, NQ), F32)))
        for t in range(-SKEW, 0):
            acc = acc + pv_tile(t)
        finish(H - 1, NJ - 1, acc, sums)

    @pl.when(jnp.logical_not(safe))
    def _():
        lax.fori_loop(0, NJ * H, shifted_body, 0)

    for cp in late_cps:
        cp.wait()
    transpose_into(wot_s, wo_v)
    column_table(2, mod_rows(2, 3))
    b_s[...] = bsp_v[...].astype(F32)
    column_table(3, 0.5 * mod_rows(3, 4))
    column_table(4, 0.5 + 0.5 * mod_rows(4, 5))
    for j in range(NJ):
        a = jnp.dot(_unpack(wot_s[zero_s[j]]), _unpack(ot_s[:, _span(j, NQ)]), preferred_element_type=F32)
        x1 = xt_s[:, _span(j, NQ)] + _lanes(mod_s[2], NQ) * a
        xt_s[:, _span(j, NQ)] = x1
        h2_s[:, _span(j, NQ)] = _layernorm(x1) * _lanes(mod_s[4], NQ) + _lanes(mod_s[3], NQ)

    transposed, win_operands = set(), {}

    def win_block(p):
        index = _span(p[0], FH // 2), _span(p[1], D // 2)
        if p not in transposed:
            transposed.add(p)
            wint_s[index] = pltpu.bitcast(win_v[index[1], _span(p[0], FH)].T, U32)
        return _unpack(wint_s[index])

    for pair in range(NJ // 2):
        seen, z2_sums = set(), {}
        for i, (a_terms, b_terms, c_terms) in enumerate(WIN_ORDER):
            if pair == 0:
                win_operands[i] = (win_block(a_terms[0][0]) if len(a_terms) == 1 else
                                   _lincomb(a_terms, lambda p: win_block(p).astype(F32)).astype(BF16))
            b = _lincomb(b_terms, lambda p: h2_s[_span(p[0], D // 2), _span(2 * pair + p[1], NQ)])
            m = jnp.dot(win_operands[i], b.astype(BF16), preferred_element_type=F32)
            for p, sign in c_terms:
                dst, cols = (z2_s if p[0] else z1_s), _span(2 * pair + p[1], NQ)
                val = _accumulate(dst[:, cols] if p in seen else None, m, sign)
                seen.add(p)
                if _pending(WIN_ORDER, i, p):
                    dst[:, cols] = val
                elif p[0]:
                    val = _gelu_of_half(val)
                    ge_s[2 * pair + p[1]][0] = val
                    z2_sums[p[1]] = jnp.sum(val.reshape(FH // 8, 8, NQ), axis=0)
                else:
                    dst[:, cols] = _gelu_of_half(val)
        for n in range(2):
            zc = ge_s[2 * pair + n][zero_s[n]] - jnp.sum(z2_sums[n], axis=0, keepdims=True) * (1.0 / FH)
            z2_s[:, _span(2 * pair + n, NQ)] = zc * lax.rsqrt(jnp.mean(zc * zc, axis=0, keepdims=True) + EPS)

    out_cps = [pltpu.make_async_copy(out_v.at[pl.ds(lo, n)], out_hbm.at[pl.ds(lo, n)], osem.at[i])
               for i, (lo, n) in enumerate(OUT_BLOCKS)]
    out_cols = [slice(lo, lo + n) for lo, n in OUT_BLOCKS]
    mb, nb = FH // 4, S // 4

    def write_out(i, y):
        res = xt_s[:, out_cols[i]] + _lanes(mod_s[5], OUT_BLOCKS[i][1]) * y
        out_v[out_cols[i], :] = res.astype(BF16).T
        out_cps[i].start()

    def project_right_half(lo, hi, acc):
        for i in range(lo, hi):
            _, b_terms, c_terms = OUT_ORDER[i]
            b = _lincomb(b_terms, lambda p: g_s[_span(p[0], KH), out_cols[p[1]]])
            m = jnp.dot(_unpack(wouta_s[i]), b.astype(BF16), preferred_element_type=F32)
            for p, sign in c_terms:
                acc[p] = _accumulate(acc.get(p), m, sign)
            for n in range(2):
                if (0, n) in acc and not any(_pending(OUT_ORDER, i, (r, n)) for r in range(2)):
                    rest = jnp.dot(_unpack(woutt_s[zero_s[n], :, 2 * KH:]), g_s[2 * KH:, out_cols[n]].astype(BF16),
                                   preferred_element_type=F32)
                    write_out(n, jnp.concatenate([acc.pop((0, n)), acc.pop((1, n))], axis=0) + rest)

    def gate(block, g):
        rows, cols = _span(block[0], mb), _span(block[1], nb)
        bias = jnp.concatenate([b_s[i:i + 1, :] for i in range(4 * block[1], 4 * block[1] + 4)], axis=1)
        y = z1_s[rows, cols] * (g + bias)
        if block[1] >= 2:
            g_s[rows, cols] = y
        else:
            y_s[_span(block[0], mb // 2), cols] = _pack(y)

    def wsp_block(p):
        return wsp_v[_span(p[1], nb), _span(p[0], nb)]

    seen, right_acc = set(), {}
    for oi, (a1, b1, c1) in enumerate(SP_OUTER):
        if len(b1) > 1:
            for r in range(2):
                for c in range(2):
                    wsum_s[oi % 2, _span(r, nb), _span(c, nb)] = _lincomb(
                        _nest(b1, [((c, r), 1)]), lambda p: wsp_block(p).astype(F32))
        seen_inner = set()
        for ii, (a2, b2, c2) in enumerate(SP_INNER):
            a = _lincomb(_nest(a1, a2), lambda p: z2_s[_span(p[0], mb), _span(p[1], nb)]).astype(BF16)
            if len(b1) > 1:
                b = _lincomb(b2, lambda p: wsum_s[oi % 2, _span(p[1], nb), _span(p[0], nb)]).astype(BF16)
            elif len(b2) > 1:
                b = _lincomb(_nest(b1, b2), lambda p: wsp_block(p).astype(F32)).astype(BF16)
            else:
                b = wsp_block(_nest(b1, b2)[0][0])
            m = lax.dot_general(a, b, NT_DIMS, preferred_element_type=F32)
            for p, sign in c2:
                index = _span(p[0], mb), _span(p[1], nb)
                val = _accumulate(macc_s[index] if p in seen_inner else None, m, sign)
                seen_inner.add(p)
                if _pending(SP_INNER, ii, p):
                    macc_s[index] = val
                    continue
                for (q, outer_sign), (block, _) in zip(c1, _nest(c1, [(p, 1)])):
                    index = _span(block[0], mb), _span(block[1], nb)
                    total = _accumulate(g_s[index] if block in seen else None, val, outer_sign)
                    seen.add(block)
                    if _pending(SP_OUTER, oi, q):
                        g_s[index] = total
                    else:
                        gate(block, total)
            if (oi, ii) == (5, 1):
                transpose_into(woutt_s, wout_v)
                column_table(5, mod_rows(5, 6))
                for i, (a_terms, _, _) in enumerate(OUT_ORDER):
                    wouta_s[i] = _pack(_lincomb(a_terms, lambda p: _unpack(
                        woutt_s[zero_s[i], _span(p[0], D // 4), _span(p[1], KH)]).astype(F32)))
                project_right_half(0, 4, right_acc)
            if (oi, ii) == (6, 1):
                project_right_half(4, 7, right_acc)
            if (oi, ii) == (6, 5):
                fences[0].wait()
    for i in range(2, len(OUT_BLOCKS)):
        y = jnp.dot(_unpack(woutt_s[zero_s[i]]), _unpack(y_s[:, out_cols[i]]), preferred_element_type=F32)
        if i == 4:
            fences[1].wait()
        write_out(i, y)
    for cp in out_cps:
        cp.wait()


_SCRATCH = [
    pltpu.VMEM((S, D), BF16),
    pltpu.VMEM((D, D), BF16),
    pltpu.VMEM((DH, D), BF16),
    pltpu.VMEM((DH, D), BF16),
    pltpu.VMEM((D, D), BF16),
    pltpu.VMEM((D, F), BF16),
    pltpu.VMEM((S, S), BF16),
    pltpu.VMEM((FH, D), BF16),
    pltpu.VMEM((D, 6 * D), BF16),
    pltpu.VMEM((S, D), BF16),
    pltpu.VMEM((6, D, 128), F32),
    pltpu.VMEM((1, D // 2 + DH, D), U32),
    pltpu.VMEM((D // 2, S), U32),
    *[pltpu.VMEM((1, 64, NQ // 2), F32)] * 2,
    pltpu.VMEM((S, DH), F32),
    pltpu.VMEM((S // 2, DH), U32),
    pltpu.VMEM((DH // 2, S), U32),
    pltpu.VMEM((VPU_OFF[-1] * 56, 8, 128), F32),
    *[pltpu.VMEM((KB // 2, NQ), U32)] * NSLOT,
    pltpu.VMEM((D, S), F32),
    pltpu.VMEM((D // 2, S), U32),
    pltpu.VMEM((1, D // 2, D), U32),
    pltpu.VMEM((F // 2, D), U32),
    pltpu.VMEM((1, D // 2, FH), U32),
    pltpu.VMEM((7, D // 4, KH), U32),
    pltpu.VMEM((D, S), F32),
    pltpu.VMEM((FH, S), F32),
    pltpu.VMEM((FH, S), F32),
    *[pltpu.VMEM((1, FH, NQ), F32)] * NJ,
    pltpu.VMEM((FH, S), F32),
    pltpu.VMEM((FH // 2, S // 2), U32),
    pltpu.VMEM((2, S // 2, S // 2), F32),
    pltpu.VMEM((FH // 2, S // 2), F32),
    pltpu.VMEM((16, 128), F32),
    pltpu.VMEM((16, 128), BF16),
    pltpu.VMEM((1, D), BF16),
    pltpu.VMEM((2, 1, D), BF16),
    pltpu.SMEM((NZERO,), jnp.int32),
    pltpu.SemaphoreType.DMA((len(X_CUTS) + 12,)),
    pltpu.SemaphoreType.DMA((len(OUT_BLOCKS),)),
]


@jax.jit
def pallas_adaLN_cond__grouped_kv_mqa__mixer_gmlp__prompt_kernel(
    A_x: jax.Array,
    A_wq: jax.Array,
    A_wk: jax.Array,
    A_wv: jax.Array,
    A_wo: jax.Array,
    B_x: jax.Array,
    B_w_in: jax.Array,
    B_w_sp: jax.Array,
    B_b_sp: jax.Array,
    B_w_out: jax.Array,
    c: jax.Array,
    w_mod: jax.Array,
):
    del B_x
    out = pl.pallas_call(
        _kernel,
        out_shape=jax.ShapeDtypeStruct((S, D), BF16),
        in_specs=[pl.BlockSpec(memory_space=pl.ANY)] * 11,
        out_specs=pl.BlockSpec(memory_space=pl.ANY),
        scratch_shapes=_SCRATCH,
        compiler_params=pltpu.CompilerParams(vmem_limit_bytes=120 * 1024 * 1024),
    )(A_x.reshape(S, D), A_wq, A_wk.T, A_wv.T, A_wo, B_w_in, B_w_sp, B_b_sp.reshape(16, 128), B_w_out, c, w_mod)
    return out.reshape(1, S, D)
```

```python
import math

import jax
import jax.numpy as jnp
from jax import lax
import jax.experimental.pallas as pl
import jax.experimental.pallas.tpu as pltpu

F32 = jnp.float32
BF16 = jnp.bfloat16
U32 = jnp.uint32

S, D, H, DH, F, FH = 2048, 512, 32, 16, 1792, 896
EPS = 1e-5
QSCALE = DH ** -0.5 * math.log2(math.e)

NQ = 512
NT = NQ // 128
NJ = S // NQ
KB = 128
NKB = S // KB
UNITS = 8
NIT = NJ * H // UNITS
LAG = 8
SAFE_BOUND = 64.0
NZERO = 64

NGROUP = S // 16
NVALU = 23
VALU_GROUPS = [p for p in range(NGROUP) if (p + 1) * NVALU // NGROUP > p * NVALU // NGROUP]
MXU_GROUPS = [p for p in range(NGROUP) if p not in VALU_GROUPS]
_ENDS = [0] + [p - g for g, p in enumerate(VALU_GROUPS)]
VALU_DUE = [lo + (hi - lo) * f - 1 for lo, hi in zip(_ENDS, _ENDS[1:]) for f in (0.27, 0.55, 0.84, 1.0)]

X_CUTS = (0, 256, 512, 896, S)
OUT_BLOCKS = ((1024, 512), (1536, 512), (0, 512), (512, 256), (768, 128), (896, 128))
KH = 384

NT_DIMS = (((1,), (1,)), ((), ()))

M1 = ([((0, 0), 1), ((1, 1), 1)], [((0, 0), 1), ((1, 1), 1)], [((0, 0), 1), ((1, 1), 1)])
M2 = ([((1, 0), 1), ((1, 1), 1)], [((0, 0), 1)], [((1, 0), 1), ((1, 1), -1)])
M3 = ([((0, 0), 1)], [((0, 1), 1), ((1, 1), -1)], [((0, 1), 1), ((1, 1), 1)])
M4 = ([((1, 1), 1)], [((1, 0), 1), ((0, 0), -1)], [((0, 0), 1), ((1, 0), 1)])
M5 = ([((0, 0), 1), ((0, 1), 1)], [((1, 1), 1)], [((0, 0), -1), ((0, 1), 1)])
M6 = ([((1, 0), 1), ((0, 0), -1)], [((0, 0), 1), ((0, 1), 1)], [((1, 1), 1)])
M7 = ([((0, 1), 1), ((1, 1), -1)], [((1, 0), 1), ((1, 1), 1)], [((0, 0), 1)])
WIN_ORDER = (M4, M2, M1, M3, M5, M6, M7)
SP_OUTER = (M3, M5, M1, M2, M6, M4, M7)
SP_INNER = (M3, M5, M1, M6, M2, M4, M7)
OUT_ORDER = (M2, M4, M1, M5, M7, M3, M6)


def _lincomb(terms, get):
    acc = None
    for p, sign in sorted(terms, key=lambda t: -t[1]):
        acc = _accumulate(acc, get(p), sign)
    return acc


def _accumulate(acc, v, sign):
    if acc is None:
        return v if sign > 0 else -v
    return acc + v if sign > 0 else acc - v


def _nest(outer, inner):
    return [((2 * p[0] + q[0], 2 * p[1] + q[1]), a * b) for p, a in outer for q, b in inner]


def _pending(products, i, block):
    return any(block == p for _, _, c in products[i + 1:] for p, _ in c)


def _layernorm(x):
    xc = x - jnp.mean(x, axis=0, keepdims=True)
    return xc * lax.rsqrt(jnp.mean(xc * xc, axis=0, keepdims=True) + EPS)


def _gelu_of_half(hx):
    c0 = 2.0 * math.sqrt(2.0 / math.pi)
    c1 = c0 * 4.0 * 0.044715
    return hx + hx * jnp.tanh(hx * (c0 + c1 * (hx * hx)))


def _pack(x):
    return pltpu.bitcast(x.astype(BF16), U32)


def _unpack(w):
    return pltpu.bitcast(w, BF16)


def _lanes(col, n):
    return jnp.concatenate([col] * (n // 128), axis=1)


def _span(i, size):
    return slice(i * size, (i + 1) * size)


def _kernel(x_hbm, wq_hbm, wkt_hbm, wvt_hbm, wo_hbm, win_hbm, wsp_hbm, bsp_hbm, wout_hbm, c_hbm, wmod_hbm,
            out_hbm,
            x_v, wq_v, wkt_v, wvt_v, wo_v, win_v, wsp_v, wout_v, wmod_v, out_v,
            mod_s, wt_s, qt_s, qtab0_s, qtab1_s, kf_s, k_s, vt_s, ktab_s, p_s, xt_s, ot_s,
            wot_s, wint_s, woutt_s, wouta_s, h2_s, z1_s, z2_s, ge0_s, ge1_s, ge2_s, ge3_s,
            g_s, y_s, wsum_s, macc_s, b_s, bsp_v, c_v, fence_v,
            zero_s, sem, osem):
    qtab_s = (qtab0_s, qtab1_s)
    ge_s = (ge0_s, ge1_s, ge2_s, ge3_s)

    copies = []

    def copy(src, dst):
        copies.append(pltpu.make_async_copy(src, dst, sem.at[len(copies)]))
        return copies[-1]

    c_cp = copy(c_hbm, c_v)
    x_cps = [copy(x_hbm.at[pl.ds(lo, hi - lo)], x_v.at[pl.ds(lo, hi - lo)]) for lo, hi in zip(X_CUTS, X_CUTS[1:])]
    wmod_a_cp = copy(wmod_hbm.at[:, pl.ds(0, 2 * D)], wmod_v.at[:, pl.ds(0, 2 * D)])
    wkt_cp = copy(wkt_hbm, wkt_v)
    wvt_cp = copy(wvt_hbm, wvt_v)
    wq_cp = copy(wq_hbm, wq_v)
    late_cps = [copy(wo_hbm, wo_v),
                copy(wmod_hbm.at[:, pl.ds(2 * D, 4 * D)], wmod_v.at[:, pl.ds(2 * D, 4 * D)]),
                copy(win_hbm, win_v), copy(bsp_hbm, bsp_v), copy(wout_hbm, wout_v), copy(wsp_hbm, wsp_v)]
    fences = [copy(c_hbm, fence_v.at[i]) for i in range(2)]
    for cp in (c_cp, x_cps[0], wmod_a_cp, wkt_cp, wvt_cp, wq_cp, *x_cps[1:], *fences):
        cp.start()

    def init_zero(i, carry):
        zero_s[i] = 0
        return carry
    lax.fori_loop(0, NZERO, init_zero, 0)

    def transpose_into(dst, src, at=0):
        for i in range(src.shape[1] // 128):
            dst[0, at + i * 64:at + (i + 1) * 64, :] = pltpu.bitcast(src[:, _span(i, 128)].T, U32)

    def mod_rows(lo, hi):
        cf = c_v[...].astype(F32)
        sc = jnp.broadcast_to(cf * jax.nn.sigmoid(cf), (16, D)).astype(BF16)
        return jnp.dot(sc, wmod_v[:, lo * D:hi * D], preferred_element_type=F32)[0:1]

    def column_table(i, row):
        mod_s[i] = jnp.broadcast_to(row, (128, D)).T

    normed, kv = {}, {}
    bounds = [jnp.zeros((8, 128), F32), jnp.zeros((1, 128), F32), jnp.zeros((DH, 128), F32)]

    def a_norm(n):
        xt = x_v[_span(n, 128), :].T.astype(F32)
        xt_s[:, _span(n, 128)] = xt
        normed[n] = _layernorm(xt)

    def a_project(n, lo, hi):
        if normed[n].dtype == F32:
            normed[n] = (normed[n] * mod_s[1] + mod_s[0]).astype(BF16)
        r = jnp.dot(_unpack(wt_s[zero_s[n], 8 * lo:8 * hi, :]), normed[n], preferred_element_type=F32)
        for i in range(max(lo, 2), hi):
            q = r[_span(i - lo, DH)] * QSCALE
            qt_s[_span(i - 2, 8), _span(n, 128)] = _pack(q)
            bounds[0] = jnp.maximum(bounds[0], q[0:8] * q[0:8] + q[8:16] * q[8:16])
        if lo == 0:
            kv[n] = r[0:2 * DH]

    def a_keys(n):
        r = kv.pop(n)
        kt = r[0:DH].astype(BF16).astype(F32)
        bounds[1] = jnp.maximum(bounds[1], jnp.sum(kt * kt, axis=0, keepdims=True))
        kf_s[_span(n, 128), :] = kt.T
        bounds[2] = jnp.maximum(bounds[2], jnp.abs(r[DH:2 * DH]))
        vt_s[:, _span(n, 128)] = r[DH:2 * DH]
        for p in range(8 * n, 8 * n + 8):
            k1, k2 = (kf_s[_span(16 * n + 15 - 2 * (p % 8) - e, 8), :] for e in range(2))
            if p in MXU_GROUPS:
                k_s[_span(MXU_GROUPS.index(p), 8), :] = _pack(jnp.concatenate([k1, k2], axis=0))
                continue
            for d in range(8):
                a11, a12, a21, a22 = (jnp.broadcast_to(k[:, e:e + 1], (8, 128)) for k in (k1, k2) for e in (d, d + 8))
                for m, v in enumerate((a11 + a22, a21 + a22, a11, a22, a11 + a12, a21 - a11, a12 - a22)):
                    ktab_s[VALU_GROUPS.index(p) * 56 + m * 8 + d] = v

    c_cp.wait()
    x_cps[0].wait()
    for n in range(X_CUTS[1] // 128):
        a_norm(n)
    wmod_a_cp.wait()
    mod_a = mod_rows(0, 2)
    column_table(0, mod_a[:, 0:D])
    column_table(1, 1.0 + mod_a[:, D:2 * D])
    wq_cp.wait()
    transpose_into(wt_s, wq_v, at=DH)
    wkt_cp.wait()
    wvt_cp.wait()
    wt_s[0, 0:8, :] = pltpu.bitcast(wkt_v[...], U32)
    wt_s[0, 8:16, :] = pltpu.bitcast(wvt_v[...], U32)
    x_cps[1].wait()
    last_tiles = [cut // 128 - 1 for cut in X_CUTS[2:]]
    for n in range(NKB):
        if n >= X_CUTS[1] // 128:
            a_norm(n)
        split = 10 if n < NKB - 2 else 26
        if n + 1 in last_tiles:
            a_project(n, 0, split)
        elif n in last_tiles:
            a_project(n, 0, 2)
            if n < NKB - 1:
                x_cps[2 + last_tiles.index(n)].wait()
            if n == last_tiles[-2]:
                for cp in late_cps:
                    cp.start()
            a_project(n - 1, split, H + 2)
            a_keys(n - 1)
            a_keys(n)
            a_project(n, 2, H + 2)
        else:
            a_project(n, 0, H + 2)
            a_keys(n)

    q2, k2, vmax = jnp.max(jnp.sum(bounds[0], axis=0, keepdims=True)), jnp.max(bounds[1]), jnp.max(bounds[2])
    safe = jnp.logical_and(q2 * k2 <= SAFE_BOUND * SAFE_BOUND, vmax <= 2.0 ** 40)

    def unit_index(h, j):
        if isinstance(h, int):
            return _span(h, 8), _span(j, NQ)
        return pl.ds(pl.multiple_of(h * 8, 8), 8), pl.ds(pl.multiple_of(j * NQ, NQ), NQ)

    def first_unit(it):
        return (it % (H // UNITS)) * UNITS, it // (H // UNITS)

    def query_table(slot, h, j):
        q = _unpack(qt_s[unit_index(h, j)]).astype(F32)
        for m in range(NT // 2):
            b11, b12, b21, b22 = (q[_span(r, 8), _span(2 * m + e, 128)] for r in range(2) for e in range(2))
            for i, v in enumerate((b11 + b22, b11, b12 - b22, b21 - b11, b22, b11 + b12, b21 + b22)):
                qtab_s[slot][0, _span(i, 8), _span(m, 128)] = v

    def times_values(t, p):
        u, kb = divmod(t, NKB)
        v = vt_s[:, pl.ds(pl.multiple_of(kb * KB + zero_s[u % NZERO] * 128, 128), KB)]
        return jnp.dot(v, p, preferred_element_type=F32)

    def finish(h, j, acc, sums):
        l = jnp.sum(sums, axis=0, keepdims=True)
        r = pl.reciprocal(l, approx=True)
        ot_s[unit_index(h, j)] = _pack(acc * (r * (2.0 - l * r)))

    def unshifted_body(it, carry):
        h0, j = first_unit(it)
        probs, sums, acc, issued, products = {}, {}, {}, {}, {}
        num_mxu = len(MXU_GROUPS)

        def valu_scores(u, g, o):
            zk, zq = zero_s[u], zero_s[2 * g]

            def product(i):
                keys = [ktab_s[g * 56 + i * 8 + d + zk] for d in range(8)]
                res = []
                for m in range(2):
                    t = [keys[d] * qtab_s[u % 2][zq, _span(8 * i + d, 1), _span(m, 128)] for d in range(8)]
                    t = [t[d] + t[d + 4] for d in range(4)]
                    res.append((t[0] + t[1]) + (t[2] + t[3]))
                return res

            def add(a, b):
                return [x + y for x, y in zip(a, b)]

            def sub(a, b):
                return [x - y for x, y in zip(a, b)]

            if o == 0:
                products[3], products[5] = product(2), product(4)
                return 0, 1, add(products[3], products[5])
            if o == 1:
                products[2], products[4] = product(1), product(3)
                return 1, 0, add(products[2], products[4])
            if o == 2:
                part = add(sub(products.pop(4), products.pop(5)), product(6))
                products[1] = product(0)
                return 0, 0, add(part, products[1])
            return 1, 1, add(add(sub(products.pop(3), products.pop(2)), products.pop(1)), product(5))

        def emit(u, group, half, n, s):
            p = jnp.exp2(s)
            sums[u, n] = p if (u, n) not in sums else sums[u, n] + p
            probs[u, group, half, n] = p

        def issue_valu(u, progress):
            while issued.get(u, 0) < len(VALU_DUE) and VALU_DUE[issued.get(u, 0)] <= progress + 1e-9:
                g, o = divmod(issued.get(u, 0), 4)
                issued[u] = issued.get(u, 0) + 1
                half, n, res = valu_scores(u, g, o)
                for m, s in enumerate(res):
                    emit(u, VALU_GROUPS[g], half, 2 * m + n, s)

        def mxu_scores(lo, hi):
            res = []
            while lo < hi:
                u, a = divmod(lo, num_mxu)
                b = min(num_mxu, a + hi - lo)
                k = k_s[pl.ds(pl.multiple_of(8 * a + zero_s[u] * 8, 8), 8 * (b - a)), :]
                rows, cols = unit_index(h0 + u, j)
                q = qt_s[pl.ds(pl.multiple_of(rows.start + zero_s[a % NZERO] * 8, 8), 8), cols]
                res.append((u, a, b, jnp.dot(_unpack(k), _unpack(q), preferred_element_type=F32)))
                lo += b - a
            return res

        def exponentiate(u, a, b, s):
            for g in range(a, b):
                for n in range(NT):
                    for e in range(2):
                        emit(u, MXU_GROUPS[g], e, n, s[_span(2 * (g - a) + e, 8), _span(n, 128)])
                    issue_valu(u, g + (n + 1) / NT)

        def tile(t):
            u, kb = divmod(t, NKB)
            return jnp.concatenate(
                [jnp.concatenate([probs.pop((u, 8 * kb + r // 2, r % 2, n)) for n in range(NT)], axis=1)
                 for r in reversed(range(16))], axis=0)

        def all_sums(u):
            return jnp.concatenate([sums[u, n] for n in range(NT)], axis=1)

        acc[-1], last_sums = carry
        pending, done = [], 0
        for t in range(UNITS * NKB):
            u, kb = divmod(t, NKB)
            upto = min(u * num_mxu + sum(p < 8 * kb for p in MXU_GROUPS) + LAG, UNITS * num_mxu)
            fresh, done = mxu_scores(done, upto), upto
            if kb == 4 and u + 1 < UNITS:
                query_table((u + 1) % 2, h0 + u + 1, j)
            elif kb == 4:
                query_table(0, *first_unit(jnp.minimum(it + 1, NIT - 1)))
            for item in pending:
                exponentiate(*item)
            pending = fresh
            d = times_values(t - 1, tile(t - 1) if t else p_s[pl.ds(pl.multiple_of(zero_s[0] * 8, 8), KB), :])
            u, kb = divmod(t - 1, NKB)
            acc[u] = pltpu.bitcast(pltpu.bitcast(d, U32), F32) if kb == 0 else acc[u] + d
            if kb == NKB - 1 and u < 0:
                h_prev, j_prev = first_unit((it + NIT - 1) % NIT)
                finish(h_prev + UNITS - 1, j_prev, acc[u], last_sums)
            elif kb == NKB - 1:
                finish(h0 + u, j, acc[u], all_sums(u))
        for item in pending:
            exponentiate(*item)
        p_s[...] = tile(UNITS * NKB - 1)
        return acc[UNITS - 1], all_sums(UNITS - 1)

    def shifted_body(it, carry):
        index = unit_index(it % H, it // H)
        s = jnp.dot(kf_s[...].astype(BF16), _unpack(qt_s[index]), preferred_element_type=F32)
        p = jnp.exp2(s - jnp.max(s, axis=0, keepdims=True))
        o = jnp.dot(vt_s[...].astype(BF16), p.astype(BF16), preferred_element_type=F32)
        ot_s[index] = _pack(o * (1.0 / jnp.sum(p, axis=0, keepdims=True)))
        return carry

    @pl.when(safe)
    def _():
        query_table(0, 0, 0)
        p_s[...] = jnp.zeros(p_s.shape, F32)
        acc, sums = lax.fori_loop(0, NIT, unshifted_body, (jnp.zeros((DH, NQ), F32), jnp.ones((8, NQ), F32)))
        finish(H - 1, NJ - 1, acc + times_values(-1, p_s[...]), sums)

    @pl.when(jnp.logical_not(safe))
    def _():
        lax.fori_loop(0, NJ * H, shifted_body, 0)

    for cp in late_cps:
        cp.wait()
    transpose_into(wot_s, wo_v)
    column_table(2, mod_rows(2, 3))
    b_s[...] = bsp_v[...].astype(F32)
    column_table(3, 0.5 * mod_rows(3, 4))
    column_table(4, 0.5 + 0.5 * mod_rows(4, 5))
    for j in range(NJ):
        a = jnp.dot(_unpack(wot_s[zero_s[j]]), _unpack(ot_s[:, _span(j, NQ)]), preferred_element_type=F32)
        x1 = xt_s[:, _span(j, NQ)] + _lanes(mod_s[2], NQ) * a
        xt_s[:, _span(j, NQ)] = x1
        h2_s[:, _span(j, NQ)] = _layernorm(x1) * _lanes(mod_s[4], NQ) + _lanes(mod_s[3], NQ)

    transposed, win_operands = set(), {}

    def win_block(p):
        index = _span(p[0], FH // 2), _span(p[1], D // 2)
        if p not in transposed:
            transposed.add(p)
            wint_s[index] = pltpu.bitcast(win_v[index[1], _span(p[0], FH)].T, U32)
        return _unpack(wint_s[index])

    for pair in range(NJ // 2):
        seen, z2_sums = set(), {}
        for i, (a_terms, b_terms, c_terms) in enumerate(WIN_ORDER):
            if pair == 0:
                win_operands[i] = (win_block(a_terms[0][0]) if len(a_terms) == 1 else
                                   _lincomb(a_terms, lambda p: win_block(p).astype(F32)).astype(BF16))
            b = _lincomb(b_terms, lambda p: h2_s[_span(p[0], D // 2), _span(2 * pair + p[1], NQ)])
            m = jnp.dot(win_operands[i], b.astype(BF16), preferred_element_type=F32)
            for p, sign in c_terms:
                dst, cols = (z2_s if p[0] else z1_s), _span(2 * pair + p[1], NQ)
                val = _accumulate(dst[:, cols] if p in seen else None, m, sign)
                seen.add(p)
                if _pending(WIN_ORDER, i, p):
                    dst[:, cols] = val
                elif p[0]:
                    val = _gelu_of_half(val)
                    ge_s[2 * pair + p[1]][0] = val
                    z2_sums[p[1]] = jnp.sum(val.reshape(FH // 8, 8, NQ), axis=0)
                else:
                    dst[:, cols] = _gelu_of_half(val)
        for n in range(2):
            zc = ge_s[2 * pair + n][zero_s[n]] - jnp.sum(z2_sums[n], axis=0, keepdims=True) * (1.0 / FH)
            z2_s[:, _span(2 * pair + n, NQ)] = zc * lax.rsqrt(jnp.mean(zc * zc, axis=0, keepdims=True) + EPS)

    out_cps = [pltpu.make_async_copy(out_v.at[pl.ds(lo, n)], out_hbm.at[pl.ds(lo, n)], osem.at[i])
               for i, (lo, n) in enumerate(OUT_BLOCKS)]
    out_cols = [slice(lo, lo + n) for lo, n in OUT_BLOCKS]
    mb, nb = FH // 4, S // 4

    def write_out(i, y):
        res = xt_s[:, out_cols[i]] + _lanes(mod_s[5], OUT_BLOCKS[i][1]) * y
        out_v[out_cols[i], :] = res.astype(BF16).T
        out_cps[i].start()

    def project_right_half(lo, hi, acc):
        for i in range(lo, hi):
            _, b_terms, c_terms = OUT_ORDER[i]
            b = _lincomb(b_terms, lambda p: g_s[_span(p[0], KH), out_cols[p[1]]])
            m = jnp.dot(_unpack(wouta_s[i]), b.astype(BF16), preferred_element_type=F32)
            for p, sign in c_terms:
                acc[p] = _accumulate(acc.get(p), m, sign)
            for n in range(2):
                if (0, n) in acc and not any(_pending(OUT_ORDER, i, (r, n)) for r in range(2)):
                    rest = jnp.dot(_unpack(woutt_s[zero_s[n], :, 2 * KH:]), g_s[2 * KH:, out_cols[n]].astype(BF16),
                                   preferred_element_type=F32)
                    write_out(n, jnp.concatenate([acc.pop((0, n)), acc.pop((1, n))], axis=0) + rest)

    def gate(block, g):
        rows, cols = _span(block[0], mb), _span(block[1], nb)
        bias = jnp.concatenate([b_s[i:i + 1, :] for i in range(4 * block[1], 4 * block[1] + 4)], axis=1)
        y = z1_s[rows, cols] * (g + bias)
        if block[1] >= 2:
            g_s[rows, cols] = y
        else:
            y_s[_span(block[0], mb // 2), cols] = _pack(y)

    def wsp_block(p):
        return wsp_v[_span(p[1], nb), _span(p[0], nb)]

    seen, right_acc = set(), {}
    for oi, (a1, b1, c1) in enumerate(SP_OUTER):
        if len(b1) > 1:
            for r in range(2):
                for c in range(2):
                    wsum_s[oi % 2, _span(r, nb), _span(c, nb)] = _lincomb(
                        _nest(b1, [((c, r), 1)]), lambda p: wsp_block(p).astype(F32))
        seen_inner = set()
        for ii, (a2, b2, c2) in enumerate(SP_INNER):
            a = _lincomb(_nest(a1, a2), lambda p: z2_s[_span(p[0], mb), _span(p[1], nb)]).astype(BF16)
            if len(b1) > 1:
                b = _lincomb(b2, lambda p: wsum_s[oi % 2, _span(p[1], nb), _span(p[0], nb)]).astype(BF16)
            elif len(b2) > 1:
                b = _lincomb(_nest(b1, b2), lambda p: wsp_block(p).astype(F32)).astype(BF16)
            else:
                b = wsp_block(_nest(b1, b2)[0][0])
            m = lax.dot_general(a, b, NT_DIMS, preferred_element_type=F32)
            for p, sign in c2:
                index = _span(p[0], mb), _span(p[1], nb)
                val = _accumulate(macc_s[index] if p in seen_inner else None, m, sign)
                seen_inner.add(p)
                if _pending(SP_INNER, ii, p):
                    macc_s[index] = val
                    continue
                for (q, outer_sign), (block, _) in zip(c1, _nest(c1, [(p, 1)])):
                    index = _span(block[0], mb), _span(block[1], nb)
                    total = _accumulate(g_s[index] if block in seen else None, val, outer_sign)
                    seen.add(block)
                    if _pending(SP_OUTER, oi, q):
                        g_s[index] = total
                    else:
                        gate(block, total)
            if (oi, ii) == (5, 1):
                transpose_into(woutt_s, wout_v)
                column_table(5, mod_rows(5, 6))
                for i, (a_terms, _, _) in enumerate(OUT_ORDER):
                    wouta_s[i] = _pack(_lincomb(a_terms, lambda p: _unpack(
                        woutt_s[zero_s[i], _span(p[0], D // 4), _span(p[1], KH)]).astype(F32)))
                project_right_half(0, 4, right_acc)
            if (oi, ii) == (6, 1):
                project_right_half(4, 7, right_acc)
            if (oi, ii) == (6, 5):
                fences[0].wait()
    for i in range(2, len(OUT_BLOCKS)):
        y = jnp.dot(_unpack(woutt_s[zero_s[i]]), _unpack(y_s[:, out_cols[i]]), preferred_element_type=F32)
        if i == 4:
            fences[1].wait()
        write_out(i, y)
    for cp in out_cps:
        cp.wait()


_SCRATCH = [
    pltpu.VMEM((S, D), BF16),
    pltpu.VMEM((D, D), BF16),
    pltpu.VMEM((DH, D), BF16),
    pltpu.VMEM((DH, D), BF16),
    pltpu.VMEM((D, D), BF16),
    pltpu.VMEM((D, F), BF16),
    pltpu.VMEM((S, S), BF16),
    pltpu.VMEM((FH, D), BF16),
    pltpu.VMEM((D, 6 * D), BF16),
    pltpu.VMEM((S, D), BF16),
    pltpu.VMEM((6, D, 128), F32),
    pltpu.VMEM((1, D // 2 + DH, D), U32),
    pltpu.VMEM((D // 2, S), U32),
    *[pltpu.VMEM((1, 64, NQ // 2), F32)] * 2,
    pltpu.VMEM((S, DH), F32),
    pltpu.VMEM((S // 2, DH), U32),
    pltpu.VMEM((DH, S), F32),
    pltpu.VMEM((NVALU * 56, 8, 128), F32),
    pltpu.VMEM((KB, NQ), F32),
    pltpu.VMEM((D, S), F32),
    pltpu.VMEM((D // 2, S), U32),
    pltpu.VMEM((1, D // 2, D), U32),
    pltpu.VMEM((F // 2, D), U32),
    pltpu.VMEM((1, D // 2, FH), U32),
    pltpu.VMEM((7, D // 4, KH), U32),
    pltpu.VMEM((D, S), F32),
    pltpu.VMEM((FH, S), F32),
    pltpu.VMEM((FH, S), F32),
    *[pltpu.VMEM((1, FH, NQ), F32)] * NJ,
    pltpu.VMEM((FH, S), F32),
    pltpu.VMEM((FH // 2, S // 2), U32),
    pltpu.VMEM((2, S // 2, S // 2), F32),
    pltpu.VMEM((FH // 2, S // 2), F32),
    pltpu.VMEM((16, 128), F32),
    pltpu.VMEM((16, 128), BF16),
    pltpu.VMEM((1, D), BF16),
    pltpu.VMEM((2, 1, D), BF16),
    pltpu.SMEM((NZERO,), jnp.int32),
    pltpu.SemaphoreType.DMA((len(X_CUTS) + 12,)),
    pltpu.SemaphoreType.DMA((len(OUT_BLOCKS),)),
]


@jax.jit
def pallas_adaLN_cond__grouped_kv_mqa__mixer_gmlp__prompt_kernel(
    A_x: jax.Array,
    A_wq: jax.Array,
    A_wk: jax.Array,
    A_wv: jax.Array,
    A_wo: jax.Array,
    B_x: jax.Array,
    B_w_in: jax.Array,
    B_w_sp: jax.Array,
    B_b_sp: jax.Array,
    B_w_out: jax.Array,
    c: jax.Array,
    w_mod: jax.Array,
):
    del B_x
    out = pl.pallas_call(
        _kernel,
        out_shape=jax.ShapeDtypeStruct((S, D), BF16),
        in_specs=[pl.BlockSpec(memory_space=pl.ANY)] * 11,
        out_specs=pl.BlockSpec(memory_space=pl.ANY),
        scratch_shapes=_SCRATCH,
        compiler_params=pltpu.CompilerParams(vmem_limit_bytes=120 * 1024 * 1024),
    )(A_x.reshape(S, D), A_wq, A_wk.T, A_wv.T, A_wo, B_w_in, B_w_sp, B_b_sp.reshape(16, 128), B_w_out, c, w_mod)
    return out.reshape(1, S, D)
```

```python
import math

import jax
import jax.numpy as jnp
from jax import lax
import jax.experimental.pallas as pl
import jax.experimental.pallas.tpu as pltpu

F32 = jnp.float32
BF16 = jnp.bfloat16
U32 = jnp.uint32

S, D, H, DH, F, FH = 2048, 512, 32, 16, 1792, 896
EPS = 1e-5
QSCALE = DH ** -0.5 * math.log2(math.e)

NQ = 512
NT = NQ // 128
NJ = S // NQ
KB = 128
NKB = S // KB
UNITS = 8
NIT = NJ * H // UNITS
LAG = 8
SAFE_BOUND = 64.0
NZERO = 64

NGROUP = S // 16
NVALU = 23
VALU_GROUPS = [p for p in range(NGROUP) if (p + 1) * NVALU // NGROUP > p * NVALU // NGROUP]
MXU_GROUPS = [p for p in range(NGROUP) if p not in VALU_GROUPS]
_ENDS = [0] + [p - g for g, p in enumerate(VALU_GROUPS)]
VALU_DUE = [lo + (hi - lo) * f - 1 for lo, hi in zip(_ENDS, _ENDS[1:]) for f in (0.27, 0.55, 0.84, 1.0)]

X_CUTS = (0, 256, 512, 896, S)
OUT_BLOCKS = ((1024, 512), (1536, 512), (0, 512), (512, 256), (768, 128), (896, 128))
KH = 384

NT_DIMS = (((1,), (1,)), ((), ()))

M1 = ([((0, 0), 1), ((1, 1), 1)], [((0, 0), 1), ((1, 1), 1)], [((0, 0), 1), ((1, 1), 1)])
M2 = ([((1, 0), 1), ((1, 1), 1)], [((0, 0), 1)], [((1, 0), 1), ((1, 1), -1)])
M3 = ([((0, 0), 1)], [((0, 1), 1), ((1, 1), -1)], [((0, 1), 1), ((1, 1), 1)])
M4 = ([((1, 1), 1)], [((1, 0), 1), ((0, 0), -1)], [((0, 0), 1), ((1, 0), 1)])
M5 = ([((0, 0), 1), ((0, 1), 1)], [((1, 1), 1)], [((0, 0), -1), ((0, 1), 1)])
M6 = ([((1, 0), 1), ((0, 0), -1)], [((0, 0), 1), ((0, 1), 1)], [((1, 1), 1)])
M7 = ([((0, 1), 1), ((1, 1), -1)], [((1, 0), 1), ((1, 1), 1)], [((0, 0), 1)])
WIN_ORDER = (M4, M2, M1, M3, M5, M6, M7)
SP_OUTER = (M3, M5, M1, M2, M6, M4, M7)
SP_INNER = (M3, M5, M1, M6, M2, M4, M7)
OUT_ORDER = (M2, M4, M1, M5, M7, M3, M6)


def _lincomb(terms, get):
    acc = None
    for p, sign in sorted(terms, key=lambda t: -t[1]):
        acc = _accumulate(acc, get(p), sign)
    return acc


def _accumulate(acc, v, sign):
    if acc is None:
        return v if sign > 0 else -v
    return acc + v if sign > 0 else acc - v


def _nest(outer, inner):
    return [((2 * p[0] + q[0], 2 * p[1] + q[1]), a * b) for p, a in outer for q, b in inner]


def _pending(products, i, block):
    return any(block == p for _, _, c in products[i + 1:] for p, _ in c)


def _layernorm(x):
    xc = x - jnp.mean(x, axis=0, keepdims=True)
    return xc * lax.rsqrt(jnp.mean(xc * xc, axis=0, keepdims=True) + EPS)


def _gelu_of_half(hx):
    c0 = 2.0 * math.sqrt(2.0 / math.pi)
    c1 = c0 * 4.0 * 0.044715
    return hx + hx * jnp.tanh(hx * (c0 + c1 * (hx * hx)))


def _pack(x):
    return pltpu.bitcast(x.astype(BF16), U32)


def _unpack(w):
    return pltpu.bitcast(w, BF16)


def _lanes(col, n):
    return jnp.concatenate([col] * (n // 128), axis=1)


def _span(i, size):
    return slice(i * size, (i + 1) * size)


def _kernel(x_hbm, wq_hbm, wkt_hbm, wvt_hbm, wo_hbm, win_hbm, wsp_hbm, bsp_hbm, wout_hbm, c_hbm, wmod_hbm,
            out_hbm,
            x_v, wq_v, wkt_v, wvt_v, wo_v, win_v, wsp_v, wout_v, wmod_v, out_v,
            mod_s, wt_s, qt_s, qtab0_s, qtab1_s, kf_s, k_s, vt_s, ktab_s, p_s, xt_s, ot_s,
            wot_s, wint_s, woutt_s, wouta_s, h2_s, z1_s, z2_s, ge0_s, ge1_s, ge2_s, ge3_s,
            g_s, y_s, wsum_s, macc_s, b_s, bsp_v, c_v, fence_v,
            zero_s, sem, osem):
    qtab_s = (qtab0_s, qtab1_s)
    ge_s = (ge0_s, ge1_s, ge2_s, ge3_s)

    copies = []

    def copy(src, dst):
        copies.append(pltpu.make_async_copy(src, dst, sem.at[len(copies)]))
        return copies[-1]

    c_cp = copy(c_hbm, c_v)
    x_cps = [copy(x_hbm.at[pl.ds(lo, hi - lo)], x_v.at[pl.ds(lo, hi - lo)]) for lo, hi in zip(X_CUTS, X_CUTS[1:])]
    wmod_a_cp = copy(wmod_hbm.at[:, pl.ds(0, 2 * D)], wmod_v.at[:, pl.ds(0, 2 * D)])
    wkt_cp = copy(wkt_hbm, wkt_v)
    wvt_cp = copy(wvt_hbm, wvt_v)
    wq_cp = copy(wq_hbm, wq_v)
    late_cps = [copy(wo_hbm, wo_v),
                copy(wmod_hbm.at[:, pl.ds(2 * D, 4 * D)], wmod_v.at[:, pl.ds(2 * D, 4 * D)]),
                copy(win_hbm, win_v), copy(bsp_hbm, bsp_v), copy(wout_hbm, wout_v), copy(wsp_hbm, wsp_v)]
    fences = [copy(c_hbm, fence_v.at[i]) for i in range(2)]
    for cp in (c_cp, x_cps[0], wmod_a_cp, wkt_cp, wvt_cp, wq_cp, *x_cps[1:], *fences):
        cp.start()

    def init_zero(i, carry):
        zero_s[i] = 0
        return carry
    lax.fori_loop(0, NZERO, init_zero, 0)

    def transpose_into(dst, src, at=0):
        for i in range(src.shape[1] // 128):
            dst[0, at + i * 64:at + (i + 1) * 64, :] = pltpu.bitcast(src[:, _span(i, 128)].T, U32)

    def mod_rows(lo, hi):
        cf = c_v[...].astype(F32)
        sc = jnp.broadcast_to(cf * jax.nn.sigmoid(cf), (16, D)).astype(BF16)
        return jnp.dot(sc, wmod_v[:, lo * D:hi * D], preferred_element_type=F32)[0:1]

    def column_table(i, row):
        mod_s[i] = jnp.broadcast_to(row, (128, D)).T

    normed, kv = {}, {}
    bounds = [jnp.zeros((8, 128), F32), jnp.zeros((1, 128), F32), jnp.zeros((DH, 128), F32)]

    def a_norm(n):
        xt = x_v[_span(n, 128), :].T.astype(F32)
        xt_s[:, _span(n, 128)] = xt
        normed[n] = _layernorm(xt)

    def a_project(n, lo, hi):
        if normed[n].dtype == F32:
            normed[n] = (normed[n] * mod_s[1] + mod_s[0]).astype(BF16)
        r = jnp.dot(_unpack(wt_s[zero_s[n], 8 * lo:8 * hi, :]), normed[n], preferred_element_type=F32)
        for i in range(max(lo, 2), hi):
            q = r[_span(i - lo, DH)] * QSCALE
            qt_s[_span(i - 2, 8), _span(n, 128)] = _pack(q)
            bounds[0] = jnp.maximum(bounds[0], q[0:8] * q[0:8] + q[8:16] * q[8:16])
        if lo == 0:
            kv[n] = r[0:2 * DH]

    def a_keys(n):
        r = kv.pop(n)
        kt = r[0:DH].astype(BF16).astype(F32)
        bounds[1] = jnp.maximum(bounds[1], jnp.sum(kt * kt, axis=0, keepdims=True))
        kf_s[_span(n, 128), :] = kt.T
        bounds[2] = jnp.maximum(bounds[2], jnp.abs(r[DH:2 * DH]))
        vt_s[:, _span(n, 128)] = r[DH:2 * DH]
        for p in range(8 * n, 8 * n + 8):
            k1, k2 = (kf_s[_span(16 * n + 15 - 2 * (p % 8) - e, 8), :] for e in range(2))
            if p in MXU_GROUPS:
                k_s[_span(MXU_GROUPS.index(p), 8), :] = _pack(jnp.concatenate([k1, k2], axis=0))
                continue
            for d in range(8):
                a11, a12, a21, a22 = (jnp.broadcast_to(k[:, e:e + 1], (8, 128)) for k in (k1, k2) for e in (d, d + 8))
                for m, v in enumerate((a11 + a22, a21 + a22, a11, a22, a11 + a12, a21 - a11, a12 - a22)):
                    ktab_s[VALU_GROUPS.index(p) * 56 + m * 8 + d] = v

    c_cp.wait()
    x_cps[0].wait()
    for n in range(X_CUTS[1] // 128):
        a_norm(n)
    wmod_a_cp.wait()
    mod_a = mod_rows(0, 2)
    column_table(0, mod_a[:, 0:D])
    column_table(1, 1.0 + mod_a[:, D:2 * D])
    wq_cp.wait()
    transpose_into(wt_s, wq_v, at=DH)
    wkt_cp.wait()
    wvt_cp.wait()
    wt_s[0, 0:8, :] = pltpu.bitcast(wkt_v[...], U32)
    wt_s[0, 8:16, :] = pltpu.bitcast(wvt_v[...], U32)
    x_cps[1].wait()
    last_tiles = [cut // 128 - 1 for cut in X_CUTS[2:]]
    for n in range(NKB):
        if n >= X_CUTS[1] // 128:
            a_norm(n)
        split = 10 if n < NKB - 2 else 26
        if n + 1 in last_tiles:
            a_project(n, 0, split)
        elif n in last_tiles:
            a_project(n, 0, 2)
            if n < NKB - 1:
                x_cps[2 + last_tiles.index(n)].wait()
            if n == last_tiles[-2]:
                for cp in late_cps:
                    cp.start()
            a_project(n - 1, split, H + 2)
            a_keys(n - 1)
            a_keys(n)
            a_project(n, 2, H + 2)
        else:
            a_project(n, 0, H + 2)
            a_keys(n)

    q2, k2, vmax = jnp.max(jnp.sum(bounds[0], axis=0, keepdims=True)), jnp.max(bounds[1]), jnp.max(bounds[2])
    safe = jnp.logical_and(q2 * k2 <= SAFE_BOUND * SAFE_BOUND, vmax <= 2.0 ** 40)

    def unit_index(h, j):
        if isinstance(h, int):
            return _span(h, 8), _span(j, NQ)
        return pl.ds(pl.multiple_of(h * 8, 8), 8), pl.ds(pl.multiple_of(j * NQ, NQ), NQ)

    def first_unit(it):
        return (it % (H // UNITS)) * UNITS, it // (H // UNITS)

    def query_table(slot, h, j):
        q = _unpack(qt_s[unit_index(h, j)]).astype(F32)
        for m in range(NT // 2):
            b11, b12, b21, b22 = (q[_span(r, 8), _span(2 * m + e, 128)] for r in range(2) for e in range(2))
            for i, v in enumerate((b11 + b22, b11, b12 - b22, b21 - b11, b22, b11 + b12, b21 + b22)):
                qtab_s[slot][0, _span(i, 8), _span(m, 128)] = v

    def times_values(t, p):
        u, kb = divmod(t, NKB)
        v = vt_s[:, pl.ds(pl.multiple_of(kb * KB + zero_s[u % NZERO] * 128, 128), KB)]
        return jnp.dot(v, p, precision=lax.Precision.DEFAULT, preferred_element_type=F32)

    def finish(h, j, acc, sums):
        l = jnp.sum(sums, axis=0, keepdims=True)
        r = pl.reciprocal(l, approx=True)
        ot_s[unit_index(h, j)] = _pack(acc * (r * (2.0 - l * r)))

    def unshifted_body(it, carry):
        h0, j = first_unit(it)
        probs, sums, acc, issued, products = {}, {}, {}, {}, {}
        num_mxu = len(MXU_GROUPS)

        def valu_scores(u, g, o):
            zk, zq = zero_s[u], zero_s[2 * g]

            def product(i):
                keys = [ktab_s[g * 56 + i * 8 + d + zk] for d in range(8)]
                res = []
                for m in range(2):
                    t = [keys[d] * qtab_s[u % 2][zq, _span(8 * i + d, 1), _span(m, 128)] for d in range(8)]
                    t = [t[d] + t[d + 4] for d in range(4)]
                    res.append((t[0] + t[1]) + (t[2] + t[3]))
                return res

            def add(a, b):
                return [x + y for x, y in zip(a, b)]

            def sub(a, b):
                return [x - y for x, y in zip(a, b)]

            if o == 0:
                products[3], products[5] = product(2), product(4)
                return 0, 1, add(products[3], products[5])
            if o == 1:
                products[2], products[4] = product(1), product(3)
                return 1, 0, add(products[2], products[4])
            if o == 2:
                part = add(sub(products.pop(4), products.pop(5)), product(6))
                products[1] = product(0)
                return 0, 0, add(part, products[1])
            return 1, 1, add(add(sub(products.pop(3), products.pop(2)), products.pop(1)), product(5))

        def emit(u, group, half, n, s):
            p = jnp.exp2(s)
            sums[u, n] = p if (u, n) not in sums else sums[u, n] + p
            probs[u, group, half, n] = p

        def issue_valu(u, progress):
            while issued.get(u, 0) < len(VALU_DUE) and VALU_DUE[issued.get(u, 0)] <= progress + 1e-9:
                g, o = divmod(issued.get(u, 0), 4)
                issued[u] = issued.get(u, 0) + 1
                half, n, res = valu_scores(u, g, o)
                for m, s in enumerate(res):
                    emit(u, VALU_GROUPS[g], half, 2 * m + n, s)

        def mxu_scores(lo, hi):
            res = []
            while lo < hi:
                u, a = divmod(lo, num_mxu)
                b = min(num_mxu, a + hi - lo)
                k = k_s[pl.ds(pl.multiple_of(8 * a + zero_s[u] * 8, 8), 8 * (b - a)), :]
                rows, cols = unit_index(h0 + u, j)
                q = qt_s[pl.ds(pl.multiple_of(rows.start + zero_s[a % NZERO] * 8, 8), 8), cols]
                res.append((u, a, b, jnp.dot(_unpack(k), _unpack(q), preferred_element_type=F32)))
                lo += b - a
            return res

        def exponentiate(u, a, b, s):
            for g in range(a, b):
                for n in range(NT):
                    for e in range(2):
                        emit(u, MXU_GROUPS[g], e, n, s[_span(2 * (g - a) + e, 8), _span(n, 128)])
                    issue_valu(u, g + (n + 1) / NT)

        def tile(t):
            u, kb = divmod(t, NKB)
            return jnp.concatenate(
                [jnp.concatenate([probs.pop((u, 8 * kb + r // 2, r % 2, n)) for n in range(NT)], axis=1)
                 for r in reversed(range(16))], axis=0)

        def all_sums(u):
            return jnp.concatenate([sums[u, n] for n in range(NT)], axis=1)

        acc[-1], last_sums = carry
        pending, done = [], 0
        for t in range(UNITS * NKB):
            u, kb = divmod(t, NKB)
            upto = min(u * num_mxu + sum(p < 8 * kb for p in MXU_GROUPS) + LAG, UNITS * num_mxu)
            fresh, done = mxu_scores(done, upto), upto
            if kb == 4 and u + 1 < UNITS:
                query_table((u + 1) % 2, h0 + u + 1, j)
            elif kb == 4:
                query_table(0, *first_unit(jnp.minimum(it + 1, NIT - 1)))
            for item in pending:
                exponentiate(*item)
            pending = fresh
            d = times_values(t - 1, tile(t - 1) if t else p_s[pl.ds(pl.multiple_of(zero_s[0] * 8, 8), KB), :])
            u, kb = divmod(t - 1, NKB)
            acc[u] = pltpu.bitcast(pltpu.bitcast(d, U32), F32) if kb == 0 else acc[u] + d
            if kb == NKB - 1 and u < 0:
                h_prev, j_prev = first_unit((it + NIT - 1) % NIT)
                finish(h_prev + UNITS - 1, j_prev, acc[u], last_sums)
            elif kb == NKB - 1:
                finish(h0 + u, j, acc[u], all_sums(u))
        for item in pending:
            exponentiate(*item)
        p_s[...] = tile(UNITS * NKB - 1)
        return acc[UNITS - 1], all_sums(UNITS - 1)

    def shifted_body(it, carry):
        index = unit_index(it % H, it // H)
        s = jnp.dot(kf_s[...].astype(BF16), _unpack(qt_s[index]), preferred_element_type=F32)
        p = jnp.exp2(s - jnp.max(s, axis=0, keepdims=True))
        o = jnp.dot(vt_s[...].astype(BF16), p.astype(BF16), preferred_element_type=F32)
        ot_s[index] = _pack(o * (1.0 / jnp.sum(p, axis=0, keepdims=True)))
        return carry

    @pl.when(safe)
    def _():
        query_table(0, 0, 0)
        p_s[...] = jnp.zeros(p_s.shape, F32)
        acc, sums = lax.fori_loop(0, NIT, unshifted_body, (jnp.zeros((DH, NQ), F32), jnp.ones((8, NQ), F32)))
        finish(H - 1, NJ - 1, acc + times_values(-1, p_s[...]), sums)

    @pl.when(jnp.logical_not(safe))
    def _():
        lax.fori_loop(0, NJ * H, shifted_body, 0)

    for cp in late_cps:
        cp.wait()
    transpose_into(wot_s, wo_v)
    column_table(2, mod_rows(2, 3))
    b_s[...] = bsp_v[...].astype(F32)
    column_table(3, 0.5 * mod_rows(3, 4))
    column_table(4, 0.5 + 0.5 * mod_rows(4, 5))
    for j in range(NJ):
        a = jnp.dot(_unpack(wot_s[zero_s[j]]), _unpack(ot_s[:, _span(j, NQ)]), preferred_element_type=F32)
        x1 = xt_s[:, _span(j, NQ)] + _lanes(mod_s[2], NQ) * a
        xt_s[:, _span(j, NQ)] = x1
        h2_s[:, _span(j, NQ)] = _layernorm(x1) * _lanes(mod_s[4], NQ) + _lanes(mod_s[3], NQ)

    transposed, win_operands = set(), {}

    def win_block(p):
        index = _span(p[0], FH // 2), _span(p[1], D // 2)
        if p not in transposed:
            transposed.add(p)
            wint_s[index] = pltpu.bitcast(win_v[index[1], _span(p[0], FH)].T, U32)
        return _unpack(wint_s[index])

    for pair in range(NJ // 2):
        seen, z2_sums = set(), {}
        for i, (a_terms, b_terms, c_terms) in enumerate(WIN_ORDER):
            if pair == 0:
                win_operands[i] = (win_block(a_terms[0][0]) if len(a_terms) == 1 else
                                   _lincomb(a_terms, lambda p: win_block(p).astype(F32)))
            b = _lincomb(b_terms, lambda p: h2_s[_span(p[0], D // 2), _span(2 * pair + p[1], NQ)])
            m = jnp.dot(win_operands[i], b.astype(win_operands[i].dtype),
                        precision=lax.Precision.DEFAULT, preferred_element_type=F32)
            for p, sign in c_terms:
                dst, cols = (z2_s if p[0] else z1_s), _span(2 * pair + p[1], NQ)
                val = _accumulate(dst[:, cols] if p in seen else None, m, sign)
                seen.add(p)
                if _pending(WIN_ORDER, i, p):
                    dst[:, cols] = val
                elif p[0]:
                    val = _gelu_of_half(val)
                    ge_s[2 * pair + p[1]][0] = val
                    z2_sums[p[1]] = jnp.sum(val.reshape(FH // 8, 8, NQ), axis=0)
                else:
                    dst[:, cols] = _gelu_of_half(val)
        for n in range(2):
            zc = ge_s[2 * pair + n][zero_s[n]] - jnp.sum(z2_sums[n], axis=0, keepdims=True) * (1.0 / FH)
            z2_s[:, _span(2 * pair + n, NQ)] = zc * lax.rsqrt(jnp.mean(zc * zc, axis=0, keepdims=True) + EPS)

    out_cps = [pltpu.make_async_copy(out_v.at[pl.ds(lo, n)], out_hbm.at[pl.ds(lo, n)], osem.at[i])
               for i, (lo, n) in enumerate(OUT_BLOCKS)]
    out_cols = [slice(lo, lo + n) for lo, n in OUT_BLOCKS]
    mb, nb = FH // 4, S // 4

    def write_out(i, y):
        res = xt_s[:, out_cols[i]] + _lanes(mod_s[5], OUT_BLOCKS[i][1]) * y
        out_v[out_cols[i], :] = res.astype(BF16).T
        out_cps[i].start()

    def project_right_half(lo, hi, acc):
        for i in range(lo, hi):
            _, b_terms, c_terms = OUT_ORDER[i]
            b = _lincomb(b_terms, lambda p: g_s[_span(p[0], KH), out_cols[p[1]]])
            m = jnp.dot(_unpack(wouta_s[i]), b.astype(BF16), preferred_element_type=F32)
            for p, sign in c_terms:
                acc[p] = _accumulate(acc.get(p), m, sign)
            for n in range(2):
                if (0, n) in acc and not any(_pending(OUT_ORDER, i, (r, n)) for r in range(2)):
                    rest = jnp.dot(_unpack(woutt_s[zero_s[n], :, 2 * KH:]), g_s[2 * KH:, out_cols[n]].astype(BF16),
                                   preferred_element_type=F32)
                    write_out(n, jnp.concatenate([acc.pop((0, n)), acc.pop((1, n))], axis=0) + rest)

    def gate(block, g):
        rows, cols = _span(block[0], mb), _span(block[1], nb)
        bias = jnp.concatenate([b_s[i:i + 1, :] for i in range(4 * block[1], 4 * block[1] + 4)], axis=1)
        y = z1_s[rows, cols] * (g + bias)
        if block[1] >= 2:
            g_s[rows, cols] = y
        else:
            y_s[_span(block[0], mb // 2), cols] = _pack(y)

    def wsp_block(p):
        return wsp_v[_span(p[1], nb), _span(p[0], nb)]

    seen, right_acc = set(), {}
    for oi, (a1, b1, c1) in enumerate(SP_OUTER):
        if len(b1) > 1:
            for r in range(2):
                for c in range(2):
                    wsum_s[oi % 2, _span(r, nb), _span(c, nb)] = _lincomb(
                        _nest(b1, [((c, r), 1)]), lambda p: wsp_block(p).astype(F32))
        seen_inner = set()
        for ii, (a2, b2, c2) in enumerate(SP_INNER):
            a = _lincomb(_nest(a1, a2), lambda p: z2_s[_span(p[0], mb), _span(p[1], nb)]).astype(BF16)
            if len(b1) > 1:
                b = _lincomb(b2, lambda p: wsum_s[oi % 2, _span(p[1], nb), _span(p[0], nb)]).astype(BF16)
            elif len(b2) > 1:
                b = _lincomb(_nest(b1, b2), lambda p: wsp_block(p).astype(F32)).astype(BF16)
            else:
                b = wsp_block(_nest(b1, b2)[0][0])
            m = lax.dot_general(a, b, NT_DIMS, preferred_element_type=F32)
            for p, sign in c2:
                index = _span(p[0], mb), _span(p[1], nb)
                val = _accumulate(macc_s[index] if p in seen_inner else None, m, sign)
                seen_inner.add(p)
                if _pending(SP_INNER, ii, p):
                    macc_s[index] = val
                    continue
                for (q, outer_sign), (block, _) in zip(c1, _nest(c1, [(p, 1)])):
                    index = _span(block[0], mb), _span(block[1], nb)
                    total = _accumulate(g_s[index] if block in seen else None, val, outer_sign)
                    seen.add(block)
                    if _pending(SP_OUTER, oi, q):
                        g_s[index] = total
                    else:
                        gate(block, total)
            if (oi, ii) == (5, 1):
                transpose_into(woutt_s, wout_v)
                column_table(5, mod_rows(5, 6))
                for i, (a_terms, _, _) in enumerate(OUT_ORDER):
                    wouta_s[i] = _pack(_lincomb(a_terms, lambda p: _unpack(
                        woutt_s[zero_s[i], _span(p[0], D // 4), _span(p[1], KH)]).astype(F32)))
                project_right_half(0, 4, right_acc)
            if (oi, ii) == (6, 1):
                project_right_half(4, 7, right_acc)
            if (oi, ii) == (6, 5):
                fences[0].wait()
    for i in range(2, len(OUT_BLOCKS)):
        y = jnp.dot(_unpack(woutt_s[zero_s[i]]), _unpack(y_s[:, out_cols[i]]), preferred_element_type=F32)
        if i == 4:
            fences[1].wait()
        write_out(i, y)
    for cp in out_cps:
        cp.wait()


_SCRATCH = [
    pltpu.VMEM((S, D), BF16),
    pltpu.VMEM((D, D), BF16),
    pltpu.VMEM((DH, D), BF16),
    pltpu.VMEM((DH, D), BF16),
    pltpu.VMEM((D, D), BF16),
    pltpu.VMEM((D, F), BF16),
    pltpu.VMEM((S, S), BF16),
    pltpu.VMEM((FH, D), BF16),
    pltpu.VMEM((D, 6 * D), BF16),
    pltpu.VMEM((S, D), BF16),
    pltpu.VMEM((6, D, 128), F32),
    pltpu.VMEM((1, D // 2 + DH, D), U32),
    pltpu.VMEM((D // 2, S), U32),
    *[pltpu.VMEM((1, 64, NQ // 2), F32)] * 2,
    pltpu.VMEM((S, DH), F32),
    pltpu.VMEM((S // 2, DH), U32),
    pltpu.VMEM((DH, S), F32),
    pltpu.VMEM((NVALU * 56, 8, 128), F32),
    pltpu.VMEM((KB, NQ), F32),
    pltpu.VMEM((D, S), F32),
    pltpu.VMEM((D // 2, S), U32),
    pltpu.VMEM((1, D // 2, D), U32),
    pltpu.VMEM((F // 2, D), U32),
    pltpu.VMEM((1, D // 2, FH), U32),
    pltpu.VMEM((7, D // 4, KH), U32),
    pltpu.VMEM((D, S), F32),
    pltpu.VMEM((FH, S), F32),
    pltpu.VMEM((FH, S), F32),
    *[pltpu.VMEM((1, FH, NQ), F32)] * NJ,
    pltpu.VMEM((FH, S), F32),
    pltpu.VMEM((FH // 2, S // 2), U32),
    pltpu.VMEM((2, S // 2, S // 2), F32),
    pltpu.VMEM((FH // 2, S // 2), F32),
    pltpu.VMEM((16, 128), F32),
    pltpu.VMEM((16, 128), BF16),
    pltpu.VMEM((1, D), BF16),
    pltpu.VMEM((2, 1, D), BF16),
    pltpu.SMEM((NZERO,), jnp.int32),
    pltpu.SemaphoreType.DMA((len(X_CUTS) + 12,)),
    pltpu.SemaphoreType.DMA((len(OUT_BLOCKS),)),
]


@jax.jit
def pallas_adaLN_cond__grouped_kv_mqa__mixer_gmlp__prompt_kernel(
    A_x: jax.Array,
    A_wq: jax.Array,
    A_wk: jax.Array,
    A_wv: jax.Array,
    A_wo: jax.Array,
    B_x: jax.Array,
    B_w_in: jax.Array,
    B_w_sp: jax.Array,
    B_b_sp: jax.Array,
    B_w_out: jax.Array,
    c: jax.Array,
    w_mod: jax.Array,
):
    del B_x
    out = pl.pallas_call(
        _kernel,
        out_shape=jax.ShapeDtypeStruct((S, D), BF16),
        in_specs=[pl.BlockSpec(memory_space=pl.ANY)] * 11,
        out_specs=pl.BlockSpec(memory_space=pl.ANY),
        scratch_shapes=_SCRATCH,
        compiler_params=pltpu.CompilerParams(vmem_limit_bytes=120 * 1024 * 1024),
    )(A_x.reshape(S, D), A_wq, A_wk.T, A_wv.T, A_wo, B_w_in, B_w_sp, B_b_sp.reshape(16, 128), B_w_out, c, w_mod)
    return out.reshape(1, S, D)
```
